```python
import os as _os
_os.environ.setdefault("JAX_PLATFORMS", "cpu")
import jax
import jax.numpy as jnp

def _softmax(x, axis=-1):
    return jax.nn.softmax(x, axis=axis)
def _gelu(x):
    return jax.nn.gelu(x, approximate=True)
def _silu(x):
    return jax.nn.silu(x)
def _sigmoid(x):
    return jax.nn.sigmoid(x)
def _layernorm(x, axis=-1, eps=1e-5):
    m = jnp.mean(x, axis=axis, keepdims=True)
    v = jnp.var(x, axis=axis, keepdims=True)
    return (x - m) / jnp.sqrt(v + eps)
def _scatter_add(tgt, idx, src, axis=0):
    return tgt.at[idx].add(src)
def _segment_sum(src, seg, n):
    return jax.ops.segment_sum(src, seg, n)
class _Rng:
    def __init__(self, key):
        self._k = key
    def _next(self):
        self._k, sub = jax.random.split(self._k)
        return sub
    def normal(self, shape):
        return jax.random.normal(self._next(), shape, dtype=jnp.bfloat16)
    def randint(self, lo, hi, shape):
        return jax.random.randint(self._next(), shape, lo, hi, dtype=jnp.int32)
    def uniform(self, shape, lo=0.0, hi=1.0):
        return jax.random.uniform(self._next(), shape, jnp.bfloat16, lo, hi)
    def permutation(self, n):
        return jax.random.permutation(self._next(), n)


kernel_name = 'gated_mix__ssm_conv_h3__linear_kernel_hedgehog__prompt'

def setup_inputs():
    _rng = _Rng(jax.random.key(int.from_bytes(__import__("os").urandom(4), "little")))
    _w = (lambda a: (lambda t: t.astype(jnp.bfloat16) if jnp.issubdtype(t.dtype, jnp.floating) else t)(jnp.asarray(a)))
    def _A_setup():
        B, S, D = 1, 2048, 576
        ks = 4
        return {
            "q": _w((lambda *s: _rng.normal(s) * 0.05)(B, S, D)),
            "k": _w((lambda *s: _rng.normal(s) * 0.4)(B, S, D)),
            "v": _w((lambda *s: _rng.normal(s) * 0.4)(B, S, D)),
            "shift_k": _w((lambda *s: _rng.normal(s) * 0.4)(D, ks) * 0.5),
            "ssm_k": _w((lambda *s: _rng.normal(s) * 0.4)(D, S) * (1.0 / S ** 0.5)),
            "ssm_D": _w((lambda *s: _rng.normal(s) * 0.4)(D)),
        }
    _A_in = _A_setup()

    def _B_setup():
        B, S, D, H = 1, 2048, 576, 32
        Dh = D // H
        return {
            "x": _w((lambda *s: _rng.normal(s) * 0.05)(B, S, D)),
            "wqkv": _w((lambda *s: _rng.normal(s) * 0.8)(D, 3 * D)),
            "w_phi": _w((lambda *s: _rng.normal(s) * 0.8)(H, Dh, Dh) * (Dh ** -0.5)),
            "wo": _w((lambda *s: _rng.normal(s) * 0.05)(D, D)),
        }
    _B_in = _B_setup()

    return {
        "A_q": _A_in["q"],
        "A_k": _A_in["k"],
        "A_v": _A_in["v"],
        "A_shift_k": _A_in["shift_k"],
        "A_ssm_k": _A_in["ssm_k"],
        "A_ssm_D": _A_in["ssm_D"],
        "B_x": _B_in["x"],
        "B_wqkv": _B_in["wqkv"],
        "B_w_phi": _B_in["w_phi"],
        "B_wo": _B_in["wo"],
        "gate_w": _w((lambda *s: _rng.normal(s) * 0.05)(576) * 16.0),
    }

def reference(A_q, A_k, A_v, A_shift_k, A_ssm_k, A_ssm_D, B_x, B_wqkv, B_w_phi, B_wo, gate_w):
    def _A_ref(q, k, v, shift_k, ssm_k, ssm_D):
        B, S, D = q.shape
        ks = shift_k.shape[-1]
        k_pad = jnp.pad(k, ((0, 0), (ks - 1, 0), (0, 0)))
        k_shift = jnp.zeros_like(k)
        for t in range(ks):
            k_shift = k_shift + k_pad[:, t:t + S, :] * shift_k[:, ks - 1 - t][None, None, :]
        kv = k_shift * v
        L = 2 * S
        kv_pad = jnp.pad(kv, ((0, 0), (0, S), (0, 0)))
        kf_pad = jnp.pad(ssm_k, ((0, 0), (0, S)))
        kv_f = (lambda x, axes=(-2,-1): jnp.fft.rfft2(x.astype(jnp.float32), axes=axes))(kv_pad[:, None, :, :], axes=(1, 2))
        kf_f = (lambda x, axes=(-2,-1): jnp.fft.rfft2(x.astype(jnp.float32), axes=axes))(kf_pad[:, None, :], axes=(1, 2))
        kf_f = (lambda x, *d: x.transpose(*d))(kf_f, 1, 2, 0)
        y_f = kv_f * kf_f[None, :, :, :]
        y = (lambda x, s, axes=(-2,-1): jnp.fft.irfft2(x, s=s, axes=axes).astype(jnp.bfloat16))(y_f, (1, L), axes=(1, 2))[:, 0, :S, :]
        y = y + kv * ssm_D[None, None, :]
        return q * y

    def _B_ref(x, wqkv, w_phi, wo):
        B, S, D = x.shape
        H = 32; Dh = D // H
        qkv = (lambda x, *d: x.transpose(*d))((x @ wqkv).reshape(B, S, 3, H, Dh), 2, 0, 3, 1, 4)
        q, k, v = qkv[0], qkv[1], qkv[2]
        pq = jnp.einsum("bhsd,hdf->bhsf", q, w_phi)
        pk = jnp.einsum("bhsd,hdf->bhsf", k, w_phi)
        phi_q = jnp.concatenate([_softmax(pq, axis=-1), _softmax(-pq, axis=-1)], axis=-1)
        phi_k = jnp.concatenate([_softmax(pk, axis=-1), _softmax(-pk, axis=-1)], axis=-1)
        kv = jnp.einsum("bhsf,bhsd->bhfd", phi_k, v)
        z  = jnp.einsum("bhsf->bhf", phi_k)
        num = jnp.einsum("bhqf,bhfd->bhqd", phi_q, kv)
        den = jnp.einsum("bhqf,bhf->bhq", phi_q, z)[..., None] + 1e-6
        o = num / den
        return (lambda x, *d: x.transpose(*d))(o, 0, 2, 1, 3).reshape(B, S, D) @ wo

    x = A_q
    g = _sigmoid((x * gate_w).sum(-1, keepdims=True))
    a = _A_ref(x, A_k, A_v, A_shift_k, A_ssm_k, A_ssm_D)
    b = _B_ref(x, B_wqkv, B_w_phi, B_wo)
    return g * a + (1 - g) * b
```

```python
import numpy as np
import jax
import jax.numpy as jnp
from jax import lax
import jax.experimental.pallas as pl
import jax.experimental.pallas.tpu as pltpu

S, D, H, DH = 2048, 576, 32, 18
T = 256
NT = S // T
CB = 64
NCB = D // CB
C = 128
NC = S // C
NG = 8
GR = 72
GX = 80
NF = 9
LOG2E = float(np.log2(np.e))
F32 = jnp.float32
BF16 = jnp.bfloat16
U32 = jnp.uint32
NT_DIMS = (((1,), (1,)), ((), ()))
HOP = 6
P = dict(c0=1300, c1=6200, s0=560, s1=1700, unroll2=1)


def _pack_np(x):
    b = np.asarray(jnp.asarray(x, BF16)).view(np.uint16).astype(np.uint32)
    return jnp.asarray(b[0::2] | (b[1::2] << 16))


def _consts():
    n = np.arange(C)[:, None].astype(np.float64)
    k = np.arange(C)[None, :].astype(np.float64)
    th = np.pi * (2 * k + 1) / (2 * C) * n
    f = np.concatenate([np.cos(th), -np.sin(th)], axis=1)
    finv = f.T / C
    col = np.arange(2 * D)
    e = ((col % D) // DH)[None, :] == np.arange(H)[:, None]
    idx = np.zeros((16, 2 * D), np.int32)
    idx[:8] = (col // DH)[None, :] - (np.arange(8) % 4)[:, None]
    idx[8:] = (col % DH)[None, :]
    t = np.arange(NF)[:, None, None]
    r = np.arange(2 * GX)[None, :, None]
    c = np.arange(128)[None, None, :]
    gr = t - 1 + r // GX
    rr = r % GX
    hr = np.where(rr < GR, rr // DH, (rr - GR) % 4)
    fi = 128 * t + c
    mask = (gr == fi // (2 * GR)) & (hr == fi % 4)
    return f, finv, e, idx, mask


def _recip(x):
    r = pl.reciprocal(x, approx=True)
    return r * (2.0 - x * r)


def _pk(x):
    return pltpu.bitcast(x.astype(BF16), U32)


def _up(x):
    return pltpu.bitcast(x, BF16)


class _Clock:
    def __init__(self, z_ref):
        self.z = z_ref
        self.v = [z_ref[0]]

    def at(self, t):
        n = int(t) // HOP
        while len(self.v) <= n:
            self.v.append(self.z[self.v[-1]])
        return self.v[n]


def _kernel(z_ref, q_h, k_h, v_h, h_h, wqkv_h, wo_h, sh_h, wp_h, dd_h, gw_h, f_h, fi_h, e_h, idx_h, msk_h,
            out_h,
            q_s, k_s, v_s, h_s, wqkv_s, wo_s, sh_s, wp_s, dd_s, gw_s, f_s, fi_s, e_s, idx_s, msk_s,
            wt_u, wot_u, tab_s, ar_s, ul_u, yb_u, yp_s, phiq_u, phik_u, vx_u, acc_s, kvm_u, ot_u, g_s, out_s,
            sem, sem_o):
    small = [(sh_h, sh_s), (wp_h, wp_s), (dd_h, dd_s), (gw_h, gw_s), (f_h, f_s), (fi_h, fi_s),
             (e_h, e_s), (idx_h, idx_s), (msk_h, msk_s)]

    def small_cp(j):
        return pltpu.make_async_copy(small[j][0], small[j][1], sem.at[j])

    def q_cp(i):
        return pltpu.make_async_copy(q_h.at[:, pl.ds(i * T, T)], q_s.at[i], sem.at[9 + i])

    def kvh_cp(b, j):
        src, dst = ((k_h, k_s), (v_h, v_s), (h_h, h_s))[j]
        return pltpu.make_async_copy(src.at[pl.ds(b * CB, CB), :], dst.at[b], sem.at[17 + 3 * b + j])

    def w_cp(j):
        src, dst = ((wqkv_h, wqkv_s), (wo_h, wo_s))[j]
        return pltpu.make_async_copy(src, dst, sem.at[44 + j])

    def o_cp(i):
        return pltpu.make_async_copy(out_s.at[i], out_h.at[:, pl.ds(i * T, T)], sem_o.at[i])

    for j in range(len(small) - 1):
        small_cp(j).start()
    for j in range(3):
        kvh_cp(0, j).start()
    w_cp(0).start()
    for j in range(3):
        kvh_cp(1, j).start()
    for i in range(NT):
        q_cp(i).start()
        if i + 2 < NCB:
            for j in range(3):
                kvh_cp(i + 2, j).start()
    w_cp(1).start()
    small_cp(8).start()

    for j in range(len(small) - 1):
        small_cp(j).wait()

    rows = [sh_s[j:j + 1, :].astype(F32) for j in range(4)]
    rows.append(dd_s[...].astype(F32).reshape(1, D))
    rows.append(gw_s[...].astype(F32).reshape(1, D))
    for j in range(6):
        tab_s[j] = jnp.broadcast_to(rows[j], (128, D)).T

    def row0(b):
        return b * CB if isinstance(b, int) else pl.multiple_of(b * CB, CB)

    def shift_conv(b, clk, t0, t1):
        lane = lax.broadcasted_iota(jnp.int32, (8, C), 1)
        m1 = lane >= 1
        m2 = lane >= 2
        r0 = row0(b)
        nstep = (CB // 8) * (NC // 2)
        for rr in range(CB // 8):
            tp = None
            p1 = p2 = None
            for ap in range(NC // 2):
                z = clk.at(t0 + (t1 - t0) * (rr * (NC // 2) + ap) / nstep)
                if tp is None:
                    tp = [tab_s[j + z, pl.ds(r0 + 8 * rr, 8), :] for j in range(4)]
                kk = k_s[b + z, 8 * rr:8 * rr + 8, ap * 2 * C:(ap + 1) * 2 * C].astype(F32)
                vv = v_s[b + z, 8 * rr:8 * rr + 8, ap * 2 * C:(ap + 1) * 2 * C].astype(F32)
                us = []
                for hf in range(2):
                    ka = kk[:, hf * C:(hf + 1) * C]
                    r1 = pltpu.roll(ka, 1, 1)
                    s1 = jnp.where(m1, r1, 0.0 if p1 is None else p1)
                    p1 = r1
                    aa = tp[0] * ka + tp[1] * s1
                    bb = tp[2] * ka + tp[3] * s1
                    r2 = pltpu.roll(bb, 2, 1)
                    s2 = jnp.where(m2, r2, 0.0 if p2 is None else p2)
                    p2 = r2
                    us.append((aa + s2) * vv[:, hf * C:(hf + 1) * C])
                o = (rr * (NC // 2) + ap) * 8
                ul_u[o:o + 8, :] = _pk(jnp.concatenate(us, axis=0))

    def fwd(b):
        lane = lax.broadcasted_iota(jnp.int32, (8, C), 1)
        sgn = jnp.where((lane & 1) == 0, 1.0, -1.0).astype(F32)
        r0 = row0(b)
        n = NC * CB
        fm = _up(f_s[...])
        r = jnp.dot(_up(ul_u[...]), fm, preferred_element_type=F32)
        ua, ub = r[:, :C], r[:, C:]
        ar_s[0, 0] = ua
        ar_s[0, 1] = ub
        ar_s[0, 2] = ua + ub
        hb = h_s[b]
        lh = jnp.concatenate([hb[:, a * C:(a + 1) * C] for a in range(NC)], axis=0)
        r = jnp.dot(lh, fm, preferred_element_type=F32)
        hre, him = r[:, :C], r[:, C:]
        sg = jnp.tile(sgn, ((n - CB) // 8, 1))
        re = jnp.concatenate([hre[:CB] + tab_s[4, pl.ds(r0, CB), :], hre[CB:] - sg * him[:n - CB]], axis=0)
        im = jnp.concatenate([him[:CB], him[CB:] + sg * hre[:n - CB]], axis=0)
        ar_s[0, 3] = re
        ar_s[0, 4] = im - re
        ar_s[0, 5] = im + re

    def cmac(clk, t0, t1):
        total = (CB // 8) * 136
        done = 0
        for rr in range(CB // 8):
            for mb in range(NC // 4):
                acc = [[None] * 3 for _ in range(4)]
                hw = {}
                for a in range(4 * mb + 4):
                    z = clk.at(t0 + (t1 - t0) * done / total)
                    o = (rr * NC + a) * 8
                    uu = [ar_s[z, j, o:o + 8, :] for j in range(3)]
                    for mi in range(4):
                        c = 4 * mb + mi - a
                        if c < 0:
                            continue
                        if c not in hw:
                            hw[c] = [ar_s[z, 3 + j, c * CB + 8 * rr:c * CB + 8 * rr + 8, :] for j in range(3)]
                        hh = hw[c]
                        prods = (uu[2] * hh[0], uu[0] * hh[1], uu[1] * hh[2])
                        done += 1
                        for j in range(3):
                            acc[mi][j] = prods[j] if acc[mi][j] is None else acc[mi][j] + prods[j]
                yre = jnp.concatenate([acc[mi][0] - acc[mi][2] for mi in range(4)], axis=0)
                yim = jnp.concatenate([acc[mi][0] + acc[mi][1] for mi in range(4)], axis=0)
                base = rr * 64 + mb * 16
                yb_u[base:base + 16, 0:C] = _pk(yre)
                yb_u[base:base + 16, C:2 * C] = _pk(yim)

    def inv(b):
        r0 = row0(b)
        y = jnp.dot(_up(yb_u[...]), _up(fi_s[...]), preferred_element_type=F32)
        cpt = T // C
        for rr in range(CB // 8):
            for m in range(NC):
                yp_s[m // cpt, pl.ds(r0 + 8 * rr, 8), (m % cpt) * C:(m % cpt + 1) * C] = (
                    y[rr * 128 + m * 8:rr * 128 + m * 8 + 8])

    dmod = idx_s[8:9, :]
    a_mat = jnp.zeros((DH, 2 * D), F32)
    for d in range(DH):
        rd = jnp.dot(wp_s[d], e_s[...], preferred_element_type=F32)
        a_mat = jnp.where(dmod == d, rd, a_mat)
    sub = lax.broadcasted_iota(jnp.int32, (8, 2 * D), 0)
    a72 = [jnp.where(sub < 4, jnp.broadcast_to(a_mat[2 * fp:2 * fp + 1], (8, 2 * D)),
                     jnp.broadcast_to(a_mat[2 * fp + 1:2 * fp + 2], (8, 2 * D))) for fp in range(9)]
    hid = idx_s[0:8, :]
    bds = []
    for g in range(16):
        lo = (g * GR) // 128 * 128
        hi = -(-((g + 1) * GR) // 128) * 128
        m = hid[:, lo:hi] == 4 * g
        bds.append(jnp.concatenate([jnp.where(m, a72[fp][:, lo:hi], 0.0) for fp in range(9)], axis=0).astype(BF16))
    acc_s[...] = jnp.zeros(acc_s.shape, F32)

    for j in range(3):
        kvh_cp(0, j).wait()
    clk = _Clock(z_ref)
    shift_conv(0, clk, 0, 0)
    fwd(0)
    cmac(clk, 0, 0)

    w_cp(0).wait()
    for j in range(3):
        kvh_cp(1, j).wait()
    clk = _Clock(z_ref)
    shift_conv(1, clk, 0, 1800)
    for sgp in range(8):
        res = []
        for g in (2 * sgp, 2 * sgp + 1):
            lo = (g * GR) // 128 * 128
            hi = -(-((g + 1) * GR) // 128) * 128
            res.append(lax.dot_general(bds[g], wqkv_s[:, lo:hi], NT_DIMS, preferred_element_type=F32))
        wt_u[sgp * GR:(sgp + 1) * GR, :] = _pk(jnp.concatenate(res, axis=0) * LOG2E)
    wt_u[D:3 * D // 2, :] = pltpu.bitcast(wqkv_s[:, 2 * D:3 * D].T, U32)

    def feature_map(p, dst, g):
        pg = p.reshape(9, 8, T)
        mx = jnp.max(pg, axis=0)
        mn = jnp.min(pg, axis=0)
        mx = jnp.maximum(mx, pltpu.roll(mx, 4, 0))
        mn = jnp.minimum(mn, pltpu.roll(mn, 4, 0))
        ep = jnp.exp2(pg - mx[None])
        en = jnp.exp2(mn[None] - pg)
        sp = jnp.sum(ep, axis=0)
        sn = jnp.sum(en, axis=0)
        sp = sp + pltpu.roll(sp, 4, 0)
        sn = sn + pltpu.roll(sn, 4, 0)
        phi = jnp.concatenate([ep * _recip(sp)[None], en * _recip(sn)[None]], axis=0)
        dst[g * GR:(g + 1) * GR, :] = _pk(phi.reshape(2 * GR, T))

    def phase1(i, carry):
        q_cp(i).wait()
        nb = jnp.minimum(i + 2, NCB - 1)

        @pl.when(i + 2 < NCB)
        def _():
            for j in range(3):
                kvh_cp(i + 2, j).wait()

        clk = _Clock(z_ref)
        fwd(i + 1)
        inv(i)
        shift_conv(nb, clk, P['s0'], P['s1'])
        cmac(clk, P['c0'], P['c1'])
        xt = q_s[i]
        for sg in range(4):
            p = jnp.dot(_up(wt_u[(4 + sg) * GR:(5 + sg) * GR, :]), xt, preferred_element_type=F32)
            feature_map(p[:GR], phik_u, 2 * sg)
            feature_map(p[GR:], phik_u, 2 * sg + 1)
        for sg in range(4):
            p = jnp.dot(_up(wt_u[sg * GR:(sg + 1) * GR, :]), xt, preferred_element_type=F32)
            feature_map(p[:GR], phiq_u.at[i], 2 * sg)
            feature_map(p[GR:], phiq_u.at[i], 2 * sg + 1)
        ones = jnp.ones((8, T), F32)
        for sg in range(4):
            vt = jnp.dot(_up(wt_u[(8 + sg) * GR:(9 + sg) * GR, :]), xt, preferred_element_type=F32)
            vx_u[sg * GX:(sg + 1) * GX, :] = _pk(jnp.concatenate([vt[:GR], ones, vt[GR:], ones], axis=0))
        for t in range(NF):
            lo = max(t - 1, 0) * GX
            hi = min(t + 1, NG) * GX
            o_lo = lo - (t - 1) * GX
            r = lax.dot_general(_up(vx_u[lo // 2:hi // 2, :]), _up(phik_u[t * 64:(t + 1) * 64, :]), NT_DIMS,
                                preferred_element_type=F32)
            acc_s[t, o_lo:o_lo + hi - lo, :] += r
        return carry

    lax.fori_loop(0, NT, phase1, 0)

    w_cp(1).wait()
    small_cp(8).wait()
    inv(NCB - 1)
    wot_u[...] = pltpu.bitcast(wo_s[...].T, U32)
    for t in range(NF):
        kvm_u[t] = _pk(acc_s[t] * msk_s[t])

    def numer(i):
        sub8 = lax.broadcasted_iota(jnp.int32, (8, T), 0)
        qf = q_s[i].astype(F32)
        gl = jnp.sum((qf * jnp.tile(tab_s[5], (1, T // 128))).reshape(D // 8, 8, T), axis=0)
        gl = gl + pltpu.roll(gl, 4, 0)
        gl = gl + pltpu.roll(gl, 2, 0)
        gl = gl + pltpu.roll(gl, 1, 0)
        gate = jax.nn.sigmoid(gl)
        g_s[i] = gate
        omg = 1.0 - gate
        rs = []
        for t in range(NF):
            lo = max(t - 1, 0) * GX
            hi = min(t + 1, NG) * GX
            o_lo = lo - (t - 1) * GX
            rs.append(jnp.dot(_up(kvm_u[t, o_lo // 2:(o_lo + hi - lo) // 2, :]),
                              _up(phiq_u[i, t * 64:(t + 1) * 64, :]), preferred_element_type=F32))
        os_ = []
        for g in range(NG):
            ng = rs[g][-GX:] + rs[g + 1][:GX]
            sc = omg * _recip(ng[GR:GX] + 1e-6)
            bc = [jnp.broadcast_to(sc[j:j + 1], (8, T)) for j in range(4)]
            pat = [bc[0], bc[0], jnp.where(sub8 < 2, bc[0], bc[1]), bc[1], jnp.where(sub8 < 4, bc[1], bc[2]),
                   bc[2], jnp.where(sub8 < 6, bc[2], bc[3]), bc[3], bc[3]]
            os_.append(ng[:GR] * jnp.concatenate(pat, axis=0))
            if g % 2 == 1:
                ot_u[i, (g // 2) * GR:(g // 2 + 1) * GR, :] = _pk(jnp.concatenate(os_, axis=0))
                os_ = []

    def final(i):
        ot = _up(ot_u[i])
        gate = g_s[i]
        for sg in range(4):
            rs = slice(sg * 2 * GR, (sg + 1) * 2 * GR)
            bt = jnp.dot(_up(wot_u[sg * GR:(sg + 1) * GR, :]), ot, preferred_element_type=F32)
            qf = q_s[i, rs, :].astype(F32)
            ga = (qf.reshape(2 * GR // 8, 8, T) * gate[None]).reshape(2 * GR, T) * yp_s[i, rs, :]
            out_s[i, rs, :] = (ga + bt).astype(BF16)
        o_cp(i).start()

    numer(0)

    if P['unroll2']:
        for i in range(NT):
            if i + 1 < NT:
                numer(i + 1)
            final(i)
    else:
        def phase2(i, carry):
            numer(jnp.minimum(i + 1, NT - 1))
            final(i)
            return carry

        lax.fori_loop(0, NT, phase2, 0)
    for i in range(NT):
        o_cp(i).wait()


@jax.jit
def pallas_gated_mix__ssm_conv_h3__linear_kernel_hedgehog__prompt_kernel(A_q, A_k, A_v, A_shift_k, A_ssm_k, A_ssm_D, B_x, B_wqkv, B_w_phi, B_wo, gate_w):
    with jax.ensure_compile_time_eval():
        f, finv, e, idx, mask = _consts()
        consts = (_pack_np(f), _pack_np(finv), jnp.asarray(e, BF16), jnp.asarray(idx), jnp.asarray(mask, F32))
    ins = (A_q[0].T, A_k[0].T, A_v[0].T, A_ssm_k, B_wqkv, B_wo, A_shift_k.T,
           B_w_phi.transpose(1, 2, 0), A_ssm_D, gate_w) + consts
    V = pltpu.VMEM
    scratch = [
        V((NT, D, T), BF16), V((NCB, CB, S), BF16), V((NCB, CB, S), BF16), V((NCB, CB, S), BF16),
        V((D, 3 * D), BF16), V((D, D), BF16),
    ] + [V(x.shape, x.dtype) for x in ins[6:]] + [
        V((3 * D // 2, D), U32), V((D // 2, D), U32), V((6, D, 128), F32),
        V((2, 6, NC * CB, C), F32), V((NC * CB // 2, C), U32), V((NC * CB // 2, 2 * C), U32),
        V((NT, D, T), F32), V((NT, D, T), U32), V((D, T), U32), V((NG * GX // 2, T), U32),
        V((NF, 2 * GX, 128), F32), V((NF, GX, 128), U32), V((NT, D // 2, T), U32), V((NT, 8, T), F32),
        V((NT, D, T), BF16),
        pltpu.SemaphoreType.DMA((46,)), pltpu.SemaphoreType.DMA((NT,)),
    ]
    out = pl.pallas_call(
        _kernel,
        in_specs=[pl.BlockSpec(memory_space=pltpu.SMEM)] + [pl.BlockSpec(memory_space=pl.ANY)] * len(ins),
        out_specs=pl.BlockSpec(memory_space=pl.ANY),
        out_shape=jax.ShapeDtypeStruct((D, S), BF16),
        scratch_shapes=scratch,
        compiler_params=pltpu.CompilerParams(vmem_limit_bytes=100 * 1024 * 1024),
        name="gm",
    )(jnp.zeros((8,), jnp.int32), *ins)
    return out.T[None]
```

```python
import functools
import numpy as np
import jax
import jax.numpy as jnp
from jax import lax
import jax.experimental.pallas as pl
import jax.experimental.pallas.tpu as pltpu

S, D, H, DH = 2048, 576, 32, 18
T = 256
NT = S // T
CB = 64
NCB = D // CB
C = 128
NC = S // C
NF = 9
PR = 17 * 8
LOG2E = float(np.log2(np.e))
EPS = 1e-6
F32 = jnp.float32
BF16 = jnp.bfloat16
U32 = jnp.uint32
NT_DIMS = (((1,), (1,)), ((), ()))
HOP = 6
P = dict(c0=1700, c1=5800, s0=560, s1=1500, ob=2, m1c0=2100, m1c1=6300, m2c0=1300, m2c1=5200,
         p3s1=1000, stop=9, split=0, vsplit=1, dep=1, seq=1, alt=0)

_H0 = [(128 * t) // 36 for t in range(NF)]
_H1 = [(128 * t + 127) // 36 for t in range(NF)]
_W0 = [(DH * h) // 8 for h in _H0]
_W1 = [-(-(DH * (h + 1)) // 8) for h in _H1]
_EXTRA = [(_W1[t] - _W0[t]) % 2 for t in range(NF)]
_NR = [8 * (_W1[t] - _W0[t] + _EXTRA[t]) for t in range(NF)]
_OFF = [sum(_NR[:t]) for t in range(NF + 1)]
_LEAD = [DH * _H0[t] - 8 * _W0[t] for t in range(NF)]
_TRAIL = [8 if _EXTRA[t] else 8 * _W1[t] - DH * (_H1[t] + 1) for t in range(NF)]
_SPLIT = [0, 1, 0, 1, 0, 1, 2, 3]


def _den_slots():
    slots = []
    for t in range(NF):
        free = list(range(_LEAD[t])) + list(range(8 - _TRAIL[t], 8))
        m = {}
        if t > 0:
            m[_H0[t]] = _SPLIT[t - 1]
        if t < NF - 1:
            m[_H1[t]] = _SPLIT[t]
        for s in m.values():
            free.remove(s)
        for h in range(_H0[t], _H1[t] + 1):
            if h not in m:
                m[h] = free.pop(0)
        slots.append(m)
    return slots


_DEN = _den_slots()


def _bf16_bits(x):
    u = np.ascontiguousarray(x, np.float32).view(np.uint32)
    return (u + 0x7FFF + ((u >> 16) & 1)) >> 16


def _pack_np(x):
    b = _bf16_bits(x)
    return (b[0::2] | (b[1::2] << 16)).astype(np.uint32)


def _consts():
    n = np.arange(C)[:, None].astype(np.float64)
    k = np.arange(C)[None, :].astype(np.float64)
    th = np.pi * (2 * k + 1) / (2 * C) * n
    f = np.concatenate([np.cos(th), -np.sin(th)], axis=1)
    finv = f.T / C
    col = np.arange(2 * D)
    e = ((col % D) // DH)[None, :] == np.arange(H)[:, None]
    idx = np.zeros((16, 2 * D), np.int32)
    idx[:8] = (col // DH)[None, :] - np.arange(8)[:, None]
    idx[8:] = (col % DH)[None, :]
    mask = np.zeros((2, _OFF[NF], 128), np.float32)
    for t in range(NF):
        fi = 128 * t + np.arange(128)
        for r in range(_NR[t]):
            g = 8 * _W0[t] + r
            if DH * _H0[t] <= g < DH * (_H1[t] + 1):
                mask[0, _OFF[t] + r] = (fi // 36 == g // DH)
        for h, s in _DEN[t].items():
            r = s if s < _LEAD[t] else _NR[t] - 8 + s
            mask[0, _OFF[t] + r] = (fi // 36 == h)
            mask[1, _OFF[t] + r] = EPS * ((fi // 36 == h) & (fi % 36 < DH))
    return _pack_np(f), _pack_np(finv), _pack_np(e), idx, mask


def _recip(x):
    r = pl.reciprocal(x, approx=True)
    return r * (2.0 - x * r)


def _pk(x):
    return pltpu.bitcast(x.astype(BF16), U32)


def _up(x):
    return pltpu.bitcast(x, BF16)


def _tree(op, xs):
    xs = list(xs)
    if P['seq'] == 1:
        return functools.reduce(op, xs)
    if P['seq'] == 2:
        return op(functools.reduce(op, xs[0::2]), functools.reduce(op, xs[1::2]))
    while len(xs) > 1:
        xs = [op(xs[i], xs[i + 1]) if i + 1 < len(xs) else xs[i] for i in range(0, len(xs), 2)]
    return xs[0]


class _Clock:
    def __init__(self, z_ref):
        self.z = z_ref
        self.v = [z_ref[0]]

    def at(self, t):
        n = int(t) // HOP
        while len(self.v) <= n:
            self.v.append(self.z[self.v[-1]])
        return self.v[n]


def _kernel(z_ref, q_h, k_h, v_h, h_h, wqkv_h, wo_h, sh_h, wp_h, dd_h, gw_h, f_h, fi_h, e_h, idx_h, msk_h,
            out_h,
            q_s, k_s, v_s, h_s, wqkv_s, wo_s, sh_s, wp_s, dd_s, gw_s, f_s, fi_s, e_s, idx_s, msk_s,
            bd_u, wt_u, wot_u, tab_s, ar_s, yb_u, yp_s, phiq_u, phik_u, vx_u, acc_s, kvm_u, ot_u, g_s, out_s,
            sem):
    def cp(src, dst, s):
        return pltpu.make_async_copy(src, dst, sem.at[s])

    def q_cp(i, s):
        return [cp(q_h.at[:, pl.ds(i * T, T)], q_s.at[i], s)]

    def row_cp(src, dst, b, s):
        return [cp(src.at[pl.ds(b * CB, CB), :], dst.at[b], s)]

    def kv_cp(b, s):
        return row_cp(k_h, k_s, b, s) + row_cp(v_h, v_s, b, s)

    def w_cp(lo, hi, s):
        return [cp(wqkv_h.at[:, pl.ds(lo, hi - lo)], wqkv_s.at[:, pl.ds(lo, hi - lo)], s)]

    S_LOOP, S_M1, S_M2, S_OUT = 3, 11, 12, 13
    grp = {
        0: lambda: [cp(a, b, 0) for a, b in ((wp_h, wp_s), (e_h, e_s), (idx_h, idx_s), (sh_h, sh_s),
                                              (dd_h, dd_s), (gw_h, gw_s))],
        1: lambda: w_cp(512, 1152, 1),
        2: lambda: q_cp(0, 2) + w_cp(0, 512, 2),
        3: lambda: w_cp(1152, 1728, 3) + kv_cp(0, 3) + [cp(f_h, f_s, 3), cp(fi_h, fi_s, 3)],
        S_M1: lambda: row_cp(h_h, h_s, 7, S_M1) + kv_cp(8, S_M1) + [cp(wo_h, wo_s, S_M1), cp(msk_h, msk_s, S_M1)],
        S_M2: lambda: row_cp(h_h, h_s, 8, S_M2),
    }

    def g_loop(i):
        return q_cp(i, S_LOOP + i) + row_cp(h_h, h_s, i - 1, S_LOOP + i) + kv_cp(i, S_LOOP + i)

    for g in range(4):
        for c in grp[g]():
            c.start()
    for i in range(1, NT):
        for c in g_loop(i):
            c.start()
    for g in (S_M1, S_M2):
        for c in grp[g]():
            c.start()

    def wait(cs):
        for c in cs:
            c.wait()

    def row0(b):
        return b * CB if isinstance(b, int) else pl.multiple_of(b * CB, CB)

    def shift_conv(b, clk, t0, t1):
        lane = lax.broadcasted_iota(jnp.int32, (8, C), 1)
        m1 = lane < C - 1
        m2 = lane < C - 2
        r0 = row0(b)
        for rr in range(CB // 8):
            tp = None
            p1 = p2 = None
            for aq in range(NC // 4):
                z = clk.at(t0 + (t1 - t0) * (rr * 4 + aq) / 32)
                if tp is None:
                    tp = [tab_s[j + z, pl.ds(r0 + 8 * rr, 8), :] for j in range(4)]
                kk = k_s[b + z, 8 * rr:8 * rr + 8, aq * 4 * C:(aq + 1) * 4 * C].astype(F32)
                vv = v_s[b + z, 8 * rr:8 * rr + 8, aq * 4 * C:(aq + 1) * 4 * C].astype(F32)
                us = []
                for hf in range(4):
                    ka = kk[:, hf * C:(hf + 1) * C]
                    s1 = pltpu.roll(jnp.where(m1, ka, 0.0 if p1 is None else p1), 1, 1)
                    p1 = ka
                    aa = tp[0] * ka + tp[1] * s1
                    bb = tp[2] * ka + tp[3] * s1
                    s2 = pltpu.roll(jnp.where(m2, bb, 0.0 if p2 is None else p2), 2, 1)
                    p2 = bb
                    us.append((aa + s2) * vv[:, hf * C:(hf + 1) * C])
                o = (rr * (NC // 4) + aq) * 8
                uu = jnp.concatenate([jnp.concatenate([us[0], us[2]], axis=1),
                                      jnp.concatenate([us[1], us[3]], axis=1)], axis=0)
                ar_s.at[0, 3][o:o + 8, :] = pltpu.bitcast(uu.astype(BF16), F32)

    def fwd(b):
        lane = lax.broadcasted_iota(jnp.int32, (8, C), 1)
        sgn = jnp.where((lane & 1) == 0, 1.0, -1.0).astype(F32)
        r0 = row0(b)
        n = NC * CB
        fm = _up(f_s[...])
        ul = _up(ar_s[0, 3, 0:n // 4, :])
        r = jnp.dot(jnp.concatenate([ul[:, :C], ul[:, C:]], axis=0), fm, preferred_element_type=F32)
        ar_s[0, 0] = r
        ar_s[0, 1, :, 0:C] = r[:, :C] + r[:, C:]
        hb = h_s[b]
        lh = jnp.concatenate([hb[:, a * C:(a + 1) * C] for a in range(NC)], axis=0)
        r = jnp.dot(lh, fm, preferred_element_type=F32)
        hre, him = r[:, :C], r[:, C:]
        sg = jnp.tile(sgn, ((n - CB) // 8, 1))
        re = jnp.concatenate([hre[:CB] + tab_s[4, pl.ds(r0, CB), :], hre[CB:] - sg * him[:n - CB]], axis=0)
        im = jnp.concatenate([him[:CB], him[CB:] + sg * hre[:n - CB]], axis=0)
        ar_s[0, 1, :, C:2 * C] = re
        ar_s[0, 2, :, 0:C] = im - re
        ar_s[0, 2, :, C:2 * C] = im + re

    def cmac(clk, t0, t1):
        total = (CB // 8) * 136
        done = 0
        ob = P['ob']
        for rr in range(CB // 8):
            for mb in range(NC // ob):
                acc = [[None] * 3 for _ in range(ob)]
                hw = {}
                for a in range(ob * mb + ob):
                    z = clk.at(t0 + (t1 - t0) * done / total)
                    o = (a % 4 // 2) * 512 + ((rr * 4 + a // 4) * 2 + a % 2) * 8
                    uu = [ar_s[z, j // 2, o:o + 8, (j % 2) * C:(j % 2 + 1) * C] for j in range(3)]
                    for mi in range(ob):
                        c = ob * mb + mi - a
                        if c < 0:
                            continue
                        if c not in hw:
                            oh = c * CB + 8 * rr
                            hw[c] = [ar_s[z, j // 2, oh:oh + 8, (j % 2) * C:(j % 2 + 1) * C] for j in range(3, 6)]
                        hh = hw[c]
                        prods = (uu[2] * hh[0], uu[0] * hh[1], uu[1] * hh[2])
                        done += 1
                        for j in range(3):
                            acc[mi][j] = prods[j] if acc[mi][j] is None else acc[mi][j] + prods[j]
                res = [jnp.concatenate([x[0] - x[2], x[0] + x[1]], axis=1) for x in acc]
                base = rr * 64 + mb * ob * 4
                yb_u[base:base + ob * 4, :] = _pk(jnp.concatenate(res, axis=0))

    def inv(b):
        r0 = row0(b)
        y = jnp.dot(_up(yb_u[...]), _up(fi_s[...]), preferred_element_type=F32)
        cpt = T // C
        for rr in range(CB // 8):
            for m in range(NC):
                yp_s[m // cpt, pl.ds(r0 + 8 * rr, 8), (m % cpt) * C:(m % cpt + 1) * C] = (
                    y[rr * 128 + m * 8:rr * 128 + m * 8 + 8])

    def fold(x):
        for gp in range(2):
            res = []
            for g in (4 * x + 2 * gp, 4 * x + 2 * gp + 1):
                lo = (g * 144) // 128 * 128
                w = lax.dot_general(_up(bd_u[g]), wqkv_s[:, lo:lo + 256], NT_DIMS, preferred_element_type=F32)
                w = w.reshape(DH, 8, D)
                res.append(((w[:DH - 1] - w[DH - 1:]) * LOG2E).reshape(PR, D))
            o = (2 * x + gp) * PR
            wt_u[o:o + PR, :] = _pk(jnp.concatenate(res, axis=0))

    def feature_map(p, dst, g, is_q):
        ps = [p[8 * f:8 * f + 8] for f in range(DH - 1)]
        mx = jnp.maximum(_tree(jnp.maximum, ps), 0.0)
        mn = jnp.minimum(_tree(jnp.minimum, ps), 0.0)
        ep = [jnp.exp2(x - mx) for x in ps] + [jnp.exp2(-mx)]
        sp = _tree(jnp.add, ep)
        if not is_q:
            rp = _recip(sp)
            ep = [x * rp for x in ep]
        for j in range(9):
            dst[pl.ds(g * 144 + j, 8, stride=DH), :] = pltpu.pack_elementwise(
                [ep[2 * j], ep[2 * j + 1]], packed_dtype=BF16)
        if P['dep'] == 1:
            mn = jnp.minimum(mn, sp)
        elif P['dep'] == 2:
            mn = jnp.minimum(mn, ep[8])
        en = [jnp.exp2(mn - x) for x in ps] + [jnp.exp2(mn)]
        rn = _recip(_tree(jnp.add, en))
        if is_q:
            rn = rn * sp
        en = [x * rn for x in en]
        for j in range(9):
            dst[pl.ds(g * 144 + 9 + j, 8, stride=DH), :] = pltpu.pack_elementwise(
                [en[2 * j], en[2 * j + 1]], packed_dtype=BF16)

    def p_piece(x, gp, n, i, xt):
        o = (2 * x + gp) * PR
        xn = xt[:, n * C:(n + 1) * C]
        dst = phik_u.at[n] if x else phiq_u.at[i, n]
        if P['split']:
            pa = jnp.dot(_up(wt_u[o:o + 72, :]), xn, preferred_element_type=F32)
            feature_map(pa[:PR], dst, 2 * gp, not x)
            pb = jnp.dot(_up(wt_u[o + 72:o + PR, :]), xn, preferred_element_type=F32)
            feature_map(jnp.concatenate([pa[PR:], pb], axis=0), dst, 2 * gp + 1, not x)
        else:
            p = jnp.dot(_up(wt_u[o:o + PR, :]), xn, preferred_element_type=F32)
            feature_map(p[:PR], dst, 2 * gp, not x)
            feature_map(p[PR:], dst, 2 * gp + 1, not x)

    def v_part(j0, j1, n, xt, held, i):
        o = 4 * PR + 4 * j0
        ex = 8 if j1 == D // 8 else 0
        vt = jnp.dot(_up(wt_u[o:o + 4 * (j1 - j0) + ex, :]), xt[:, n * C:(n + 1) * C], preferred_element_type=F32)
        if ex:
            g_s[i, :, n * C:(n + 1) * C] = jax.nn.sigmoid(vt[8 * (j1 - j0):8 * (j1 - j0) + 8])
        for j in range(j0, j1):
            held[j] = vt[8 * (j - j0):8 * (j - j0) + 8]
        sub = lax.broadcasted_iota(jnp.int32, (8, C), 0)
        for t in range(NF):
            if not (j0 < _W1[t] <= j1):
                continue
            rows = [held[j] for j in range(_W0[t], _W1[t])]
            if _LEAD[t]:
                rows[0] = jnp.where(sub < _LEAD[t], 1.0, rows[0])
            if _EXTRA[t]:
                rows.append(jnp.ones((8, C), F32))
            elif _TRAIL[t]:
                rows[-1] = jnp.where(sub >= 8 - _TRAIL[t], 1.0, rows[-1])
            vx_u[_OFF[t] // 2:_OFF[t + 1] // 2, n * C:(n + 1) * C] = _pk(jnp.concatenate(rows, axis=0))

    def v_piece(hf, n, xt, held, i):
        if P['vsplit']:
            v_part(36 * hf, 36 * hf + 18, n, xt, held, i)
            v_part(36 * hf + 18, 36 * hf + 36, n, xt, held, i)
        else:
            v_part(36 * hf, 36 * hf + 36, n, xt, held, i)

    def kv_acc():
        for t in range(NF):
            ph = jnp.concatenate([_up(phik_u[n, t * 64:(t + 1) * 64, :]) for n in range(2)], axis=1)
            r = lax.dot_general(_up(vx_u[_OFF[t] // 2:_OFF[t + 1] // 2, :]), ph, NT_DIMS,
                                preferred_element_type=F32)
            acc_s[_OFF[t]:_OFF[t + 1], :] += r

    def numer(i):
        sub = lax.broadcasted_iota(jnp.int32, (8, T), 0)
        omg = 1.0 - g_s[i]
        rs = []
        for t in range(NF):
            ph = jnp.concatenate([_up(phiq_u[i, n, t * 64:(t + 1) * 64, :]) for n in range(2)], axis=1)
            rs.append(jnp.dot(_up(kvm_u[_OFF[t] // 2:_OFF[t + 1] // 2, 0:128]), ph, preferred_element_type=F32))
        es = []
        for t in range(NF):
            first, last = rs[t][0:8], rs[t][_NR[t] - 8:]
            if _LEAD[t] and _TRAIL[t]:
                es.append(jnp.where(sub < _LEAD[t], first, last))
            else:
                es.append(first if _LEAD[t] else last)
        bc = {}
        for t in range(NF):
            den = es[t] if t == NF - 1 else es[t] + jnp.where(sub == _SPLIT[t], es[t + 1], 0.0)
            sc = omg * _recip(den)
            for h, s in _DEN[t].items():
                if t == 0 or h != _H0[t]:
                    bc[h] = jnp.broadcast_to(sc[s:s + 1], (8, T))
        outs = []
        for j in range(D // 8):
            parts = []
            for t in range(NF):
                if _W0[t] <= j < _W1[t]:
                    x = rs[t][8 * (j - _W0[t]):8 * (j - _W0[t]) + 8]
                    if j == _W0[t] and _LEAD[t]:
                        x = jnp.where(sub < _LEAD[t], 0.0, x)
                    if j == _W1[t] - 1 and _TRAIL[t] and not _EXTRA[t]:
                        x = jnp.where(sub >= 8 - _TRAIL[t], 0.0, x)
                    parts.append(x)
            num = parts[0] if len(parts) == 1 else parts[0] + parts[1]
            ha, hb = (8 * j) // DH, (8 * j + 7) // DH
            sc = bc[ha] if ha == hb else jnp.where(sub < DH * hb - 8 * j, bc[ha], bc[hb])
            outs.append(num * sc)
            if j % 18 == 17:
                ot_u.at[i][(j // 18) * 72:(j // 18 + 1) * 72, :] = _pk(jnp.concatenate(outs, axis=0))
                outs = []

    def final(sg, i):
        rs = slice(sg * 144, (sg + 1) * 144)
        bt = jnp.dot(_up(wot_u[sg * 72:(sg + 1) * 72, :]), _up(ot_u[i]), preferred_element_type=F32)
        qf = q_s[i, rs, :].astype(F32)
        ga = (qf.reshape(18, 8, T) * g_s[i][None]).reshape(144, T) * yp_s[i, rs, :]
        out_s[rs, i * T:(i + 1) * T] = (ga + bt).astype(BF16)

    def o_cp(sg, i0, i1, nsg):
        sl = (pl.ds(sg * 144, nsg * 144), pl.ds(i0 * T, (i1 - i0) * T))
        return cp(out_s.at[sl], out_h.at[sl], S_OUT)

    wait(grp[0]())
    dmod = idx_s[8:9, :]
    a_mat = jnp.zeros((DH, 2 * D), F32)
    em = _up(e_s[...])
    for d in range(DH):
        rd = jnp.dot(wp_s[d], em, preferred_element_type=F32)
        a_mat = jnp.where(dmod == d, rd, a_mat)
    ab = [jnp.broadcast_to(a_mat[f:f + 1], (8, 2 * D)) for f in range(DH)]
    hid = idx_s[0:8, :]
    for g in (4, 5, 6, 7, 0, 1, 2, 3):
        lo = (g * 144) // 128 * 128
        m = hid[:, lo:lo + 256] == 8 * g
        bd_u.at[g][...] = _pk(jnp.concatenate([jnp.where(m, ab[f][:, lo:lo + 256], 0.0) for f in range(DH)], axis=0))
    acc_s[...] = jnp.zeros(acc_s.shape, F32)
    yb_u[...] = jnp.zeros(yb_u.shape, U32)

    rows = [sh_s[j:j + 1, :].astype(F32) for j in range(4)]
    rows.append(dd_s[...].astype(F32).reshape(1, D))
    wt_u[4 * PR + D // 2:4 * PR + D // 2 + 8, :] = _pk(
        jnp.broadcast_to(gw_s[...].astype(F32).reshape(1, D), (16, D)))
    for j in range(5):
        tab_s[j] = jnp.broadcast_to(rows[j], (128, D)).T

    wait(grp[1]())
    fold(1)

    wait(grp[2]())
    xt = q_s[0]
    for gp in range(2):
        for n in range(2):
            p_piece(1, gp, n, 0, xt)
    fold(0)

    wait(grp[3]())
    shift_conv(0, _Clock(z_ref), 0, P['p3s1'])
    wt_u[4 * PR:4 * PR + D // 2, :] = pltpu.bitcast(wqkv_s[:, 2 * D:3 * D].T, U32)
    xt = q_s[0]
    for gp in range(2):
        for n in range(2):
            p_piece(0, gp, n, 0, xt)
    for n in range(2):
        held = {}
        for hf in range(2):
            v_piece(hf, n, xt, held, 0)

    def phase1(i, carry):
        wait(g_loop(i))
        clk = _Clock(z_ref)
        fwd(i - 1)
        inv(jnp.maximum(i - 2, 0))
        kv_acc()
        shift_conv(i, clk, P['s0'], P['s1'])
        cmac(clk, P['c0'], P['c1'])
        xt = q_s[i]
        for n in range(2):
            held = {}
            for gp in range(2):
                if P['alt']:
                    p_piece(1, gp, n, i, xt)
                    v_part(36 * gp, 36 * gp + 18, n, xt, held, i)
                    p_piece(0, gp, n, i, xt)
                    v_part(36 * gp + 18, 36 * gp + 36, n, xt, held, i)
                else:
                    p_piece(1, gp, n, i, xt)
                    p_piece(0, gp, n, i, xt)
                    v_piece(gp, n, xt, held, i)
        return carry

    lax.fori_loop(1, NT, phase1, 0)
    if P['stop'] == 1:
        wait(grp[S_M1]() + grp[S_M2]())
        for r in (phiq_u, acc_s, yp_s, yb_u, g_s, phik_u, vx_u, ar_s):
            c = cp(r, r, S_OUT)

            @pl.when(z_ref[0] == 1)
            def _(c=c):
                c.start()
                c.wait()
        return

    wait(grp[S_M1]())
    clk = _Clock(z_ref)
    kv_acc()
    fwd(7)
    inv(6)
    shift_conv(8, clk, P['s0'] + 400, P['m1c0'] - 200)
    cmac(clk, P['m1c0'], P['m1c1'])
    wot_u[...] = pltpu.bitcast(wo_s[...].T, U32)
    kvm_u[:, 0:128] = _pk(acc_s[...] * msk_s[0] + msk_s[1])
    numer(0)
    for i in range(4):
        numer(i + 1)
        final(0, i)
        final(1, i)

    wait(grp[S_M2]())
    clk = _Clock(z_ref)
    fwd(8)
    inv(7)
    cmac(clk, P['m2c0'], P['m2c1'])
    o_cp(0, 0, 4, 2).start()
    for i in range(4, NT):
        if i + 1 < NT:
            numer(i + 1)
        final(0, i)
        final(1, i)

    o_cp(0, 0, 4, 2).wait()
    outs = [(0, 4, NT, 2)]
    o_cp(*outs[-1]).start()
    final(2, 0)
    inv(8)
    for sg, i in [(sg, i) for sg in (2, 3) for i in range(NT)][1:]:
        final(sg, i)
        if sg < 3 and i == NT - 1:
            outs.append((sg, 0, NT, 1))
            o_cp(*outs[-1]).start()
        elif sg == 3 and i in (3, 5, 6, 7):
            outs.append((sg, {3: 0, 5: 4, 6: 6, 7: 7}[i], i + 1, 1))
            o_cp(*outs[-1]).start()
    for o in outs:
        o_cp(*o).wait()


@jax.jit
def pallas_gated_mix__ssm_conv_h3__linear_kernel_hedgehog__prompt_kernel(A_q, A_k, A_v, A_shift_k, A_ssm_k, A_ssm_D, B_x, B_wqkv, B_w_phi, B_wo, gate_w):
    ins = (A_q[0].T, A_k[0].T, A_v[0].T, A_ssm_k, B_wqkv, B_wo, A_shift_k.T,
           B_w_phi.transpose(1, 2, 0), A_ssm_D, gate_w) + _consts()
    V = pltpu.VMEM
    scratch = [
        V((NT, D, T), BF16), V((NCB, CB, S), BF16), V((NCB, CB, S), BF16), V((NCB, CB, S), BF16),
        V((D, 3 * D), BF16), V((D, D), BF16),
    ] + [V(x.shape, x.dtype) for x in ins[6:]] + [
        V((8, 72, 256), U32), V((4 * PR + D // 2 + 8, D), U32), V((D // 2, D), U32), V((5, D, 128), F32),
        V((2, 4, NC * CB, 2 * C), F32), V((NC * CB // 2, 2 * C), U32),
        V((NT, D, T), F32), V((NT, 2, D, C), U32), V((2, D, C), U32), V((_OFF[NF] // 2, T), U32),
        V((_OFF[NF], 128), F32), V((_OFF[NF] // 2, 256), U32), V((NT, D // 2, T), U32), V((NT, 8, T), F32),
        V((D, S), BF16),
        pltpu.SemaphoreType.DMA((14,)),
    ]
    out = pl.pallas_call(
        _kernel,
        in_specs=[pl.BlockSpec(memory_space=pltpu.SMEM)] + [pl.BlockSpec(memory_space=pl.ANY)] * len(ins),
        out_specs=pl.BlockSpec(memory_space=pl.ANY),
        out_shape=jax.ShapeDtypeStruct((D, S), BF16),
        scratch_shapes=scratch,
        compiler_params=pltpu.CompilerParams(vmem_limit_bytes=100 * 1024 * 1024),
        name="gm",
    )(np.zeros((8,), np.int32), *ins)
    return out.T[None]
```

```python
import functools
import numpy as np
import jax
import jax.numpy as jnp
from jax import lax
import jax.experimental.pallas as pl
import jax.experimental.pallas.tpu as pltpu

S, D, H, DH = 2048, 576, 32, 18
T = 256
NT = S // T
CB = 64
NCB = D // CB
C = 128
NC = S // C
NF = 9
PR = 17 * 8
LOG2E = float(np.log2(np.e))
EPS = 1e-6
F32 = jnp.float32
BF16 = jnp.bfloat16
U32 = jnp.uint32
NT_DIMS = (((1,), (1,)), ((), ()))
HOP = 6
P = dict(c0=1250, c1=5300, s0=560, s1=1500, ob=2, m1c0=1300, m1c1=5600, m2c0=1300, m2c1=5200,
         p3s1=1000, stop=9, split=0, vsplit=1, dep=1, seq=1, alt=0, i1c0=1300, i1c1=3500, opq=1, sep=1, i1s0=560, i1s1=1500, m1s0=560, m1s1=1500, aft=0, wr=35, w0=2400, wl=600, wp=1075)

_H0 = [(128 * t) // 36 for t in range(NF)]
_H1 = [(128 * t + 127) // 36 for t in range(NF)]
_W0 = [(DH * h) // 8 for h in _H0]
_W1 = [-(-(DH * (h + 1)) // 8) for h in _H1]
_EXTRA = [(_W1[t] - _W0[t]) % 2 for t in range(NF)]
_NR = [8 * (_W1[t] - _W0[t] + _EXTRA[t]) for t in range(NF)]
_OFF = [sum(_NR[:t]) for t in range(NF + 1)]
_LEAD = [DH * _H0[t] - 8 * _W0[t] for t in range(NF)]
_TRAIL = [8 if _EXTRA[t] else 8 * _W1[t] - DH * (_H1[t] + 1) for t in range(NF)]
_SPLIT = [0, 1, 0, 1, 0, 1, 2, 3]


def _den_slots():
    slots = []
    for t in range(NF):
        free = list(range(_LEAD[t])) + list(range(8 - _TRAIL[t], 8))
        m = {}
        if t > 0:
            m[_H0[t]] = _SPLIT[t - 1]
        if t < NF - 1:
            m[_H1[t]] = _SPLIT[t]
        for s in m.values():
            free.remove(s)
        for h in range(_H0[t], _H1[t] + 1):
            if h not in m:
                m[h] = free.pop(0)
        slots.append(m)
    return slots


_DEN = _den_slots()


def _bf16_bits(x):
    u = np.ascontiguousarray(x, np.float32).view(np.uint32)
    return (u + 0x7FFF + ((u >> 16) & 1)) >> 16


def _pack_np(x):
    b = _bf16_bits(x)
    return (b[0::2] | (b[1::2] << 16)).astype(np.uint32)


def _consts():
    n = np.arange(C)[:, None].astype(np.float64)
    k = np.arange(C)[None, :].astype(np.float64)
    th = np.pi * (2 * k + 1) / (2 * C) * n
    f = np.concatenate([np.cos(th), -np.sin(th)], axis=1)
    finv = f.T / C
    mask = np.zeros((2, _OFF[NF], 128), np.float32)
    for t in range(NF):
        fi = 128 * t + np.arange(128)
        for r in range(_NR[t]):
            g = 8 * _W0[t] + r
            if DH * _H0[t] <= g < DH * (_H1[t] + 1):
                mask[0, _OFF[t] + r] = (fi // 36 == g // DH)
        for h, s in _DEN[t].items():
            r = s if s < _LEAD[t] else _NR[t] - 8 + s
            mask[0, _OFF[t] + r] = (fi // 36 == h)
            mask[1, _OFF[t] + r] = EPS * ((fi // 36 == h) & (fi % 36 < DH))
    return _pack_np(f), _pack_np(finv), mask


def _recip(x):
    r = pl.reciprocal(x, approx=True)
    return r * (2.0 - x * r)


def _pk(x):
    return pltpu.bitcast(x.astype(BF16), U32)


def _up(x):
    return pltpu.bitcast(x, BF16)


def _tree(op, xs):
    xs = list(xs)
    if P['seq'] == 1:
        return functools.reduce(op, xs)
    if P['seq'] == 2:
        return op(functools.reduce(op, xs[0::2]), functools.reduce(op, xs[1::2]))
    while len(xs) > 1:
        xs = [op(xs[i], xs[i + 1]) if i + 1 < len(xs) else xs[i] for i in range(0, len(xs), 2)]
    return xs[0]


def _warp(t0, t1, slow):
    ts = np.arange(t0, t1 + 1)
    rate = np.ones(len(ts))
    for a, b in slow:
        rate[(ts >= a) & (ts < b)] = P['wr'] / 100
    cum = np.cumsum(rate)
    return lambda fr: ts[min(int(np.searchsorted(cum, fr * cum[-1])), len(ts) - 1)]


class _Clock:
    def __init__(self, z_ref):
        self.z = z_ref
        self.v = [z_ref[0]]

    def at(self, t):
        n = int(t) // HOP
        while len(self.v) <= n:
            self.v.append(self.z[self.v[-1]])
        return self.v[n]


def _kernel(z_h, q_h, k_h, v_h, h_h, wqkv_h, wo_h, sh_h, wp_h, dd_h, gw_h, f_h, fi_h, msk_h,
            out_h,
            q_s, k_s, v_s, h_s, wqkv_s, wo_s, ar_s, tab_s, yb_u, yp_s, phiq_u, phik_u, ot_u, g_s, out_s, ul_s,
            bd_u, wot_u, wt_u, vx_u, acc_s, kvm_u,
            sh_s, wp_s, dd_s, gw_s, f_s, fi_s, msk_s, r4_s,
            z_ref, sem):
    def cp(src, dst, s):
        return pltpu.make_async_copy(src, dst, sem.at[s])

    def q_cp(i, s):
        return [cp(q_h.at[:, pl.ds(i * T, T)], q_s.at[i], s)]

    def row_cp(src, dst, b, s):
        return [cp(src.at[pl.ds(b * CB, CB), :], dst.at[b], s)]

    def kv_cp(b, s):
        return row_cp(k_h, k_s, b, s) + row_cp(v_h, v_s, b, s)

    def w_cp(lo, hi, s):
        return [cp(wqkv_h.at[:, pl.ds(lo, hi - lo)], wqkv_s.at[:, pl.ds(lo, hi - lo)], s)]

    S_LOOP, S_M1, S_M2, S_OUT = 3, 11, 12, 13
    grp = {
        0: lambda: [cp(a, b, 0) for a, b in ((wp_h, wp_s), (sh_h, sh_s), (dd_h, dd_s), (gw_h, gw_s))],
        1: lambda: w_cp(512, 1152, 1),
        2: lambda: q_cp(0, 2) + q_cp(1, 2),
        3: lambda: w_cp(0, 512, 3) + kv_cp(0, 3) + [cp(z_h, z_ref, 3)],
        4: lambda: (w_cp(1152, 1728, 4) + [cp(f_h, f_s, 4)] + row_cp(h_h, h_s, 0, 4) + kv_cp(1, 4)
                    + [cp(fi_h, fi_s, 4)]),
        S_M1: lambda: row_cp(h_h, h_s, 7, S_M1) + kv_cp(8, S_M1) + [cp(wo_h, wo_s, S_M1), cp(msk_h, msk_s, S_M1)],
        S_M2: lambda: row_cp(h_h, h_s, 8, S_M2),
    }

    def g_loop(i):
        return q_cp(i, S_LOOP + i) + row_cp(h_h, h_s, i - 1, S_LOOP + i) + kv_cp(i, S_LOOP + i)

    for g in range(5):
        for c in grp[g]():
            c.start()
    for i in range(2, NT):
        for c in g_loop(i):
            c.start()
    for g in (S_M1, S_M2):
        for c in grp[g]():
            c.start()

    def wait(cs):
        for c in cs:
            c.wait()

    def row0(b):
        return b * CB if isinstance(b, int) else pl.multiple_of(b * CB, CB)

    def shift_conv(b, clk, t0, t1):
        lane = lax.broadcasted_iota(jnp.int32, (8, C), 1)
        m1 = lane < C - 1
        m2 = lane < C - 2
        r0 = row0(b)
        zf = z_ref[1].astype(F32)
        for rr in range(CB // 8):
            tp = None
            p1 = p2 = None
            for aq in range(NC // 4):
                z = clk.at(t0 + (t1 - t0) * (rr * 4 + aq) / 32)
                if tp is None:
                    tp = [tab_s[j + z, pl.ds(r0 + 8 * rr, 8), :] for j in range(4)]
                kk = k_s[b + z, 8 * rr:8 * rr + 8, aq * 4 * C:(aq + 1) * 4 * C].astype(F32)
                vv = v_s[b + z, 8 * rr:8 * rr + 8, aq * 4 * C:(aq + 1) * 4 * C].astype(F32)
                us = []
                for hf in range(4):
                    ka = kk[:, hf * C:(hf + 1) * C]
                    c1 = jnp.where(m1, ka, 0.0 if p1 is None else p1)
                    if P['opq']:
                        c1 = c1 + zf
                    s1 = pltpu.roll(c1, 1, 1)
                    p1 = ka
                    aa = tp[0] * ka + tp[1] * s1
                    bb = tp[2] * ka + tp[3] * s1
                    s2 = pltpu.roll(jnp.where(m2, bb, 0.0 if p2 is None else p2), 2, 1)
                    p2 = bb
                    us.append((aa + s2) * vv[:, hf * C:(hf + 1) * C])
                o = (rr * (NC // 4) + aq) * 8
                uu = jnp.concatenate([jnp.concatenate([us[0], us[2]], axis=1),
                                      jnp.concatenate([us[1], us[3]], axis=1)], axis=0)
                (ul_s if P['sep'] else ar_s.at[0, 3])[o:o + 8, :] = pltpu.bitcast(uu.astype(BF16), F32)

    def fwd(b):
        lane = lax.broadcasted_iota(jnp.int32, (8, C), 1)
        sgn = jnp.where((lane & 1) == 0, 1.0, -1.0).astype(F32)
        r0 = row0(b)
        n = NC * CB
        fm = _up(f_s[...])
        ul = _up(ul_s[...] if P['sep'] else ar_s[0, 3, 0:n // 4, :])
        r = jnp.dot(jnp.concatenate([ul[:, :C], ul[:, C:]], axis=0), fm, preferred_element_type=F32)
        ar_s[0, 0] = r
        ar_s[0, 1, :, 0:C] = r[:, :C] + r[:, C:]
        hb = h_s[b]
        lh = jnp.concatenate([hb[:, a * C:(a + 1) * C] for a in range(NC)], axis=0)
        r = jnp.dot(lh, fm, preferred_element_type=F32)
        hre, him = r[:, :C], r[:, C:]
        sg = jnp.tile(sgn, ((n - CB) // 8, 1))
        re = jnp.concatenate([hre[:CB] + tab_s[4, pl.ds(r0, CB), :], hre[CB:] - sg * him[:n - CB]], axis=0)
        im = jnp.concatenate([him[:CB], him[CB:] + sg * hre[:n - CB]], axis=0)
        ar_s[0, 1, :, C:2 * C] = re
        ar_s[0, 2, :, 0:C] = im - re
        ar_s[0, 2, :, C:2 * C] = im + re

    def cmac(clk, t0, t1, slow=()):
        tm = _warp(t0, t1, slow)
        total = (CB // 8) * 136
        done = 0
        ob = P['ob']
        for rr in range(CB // 8):
            for mb in range(NC // ob):
                acc = [[None] * 3 for _ in range(ob)]
                hw = {}
                for a in range(ob * mb + ob):
                    z = clk.at(tm(done / total))
                    o = (a % 4 // 2) * 512 + ((rr * 4 + a // 4) * 2 + a % 2) * 8
                    uu = [ar_s[z, j // 2, o:o + 8, (j % 2) * C:(j % 2 + 1) * C] for j in range(3)]
                    for mi in range(ob):
                        c = ob * mb + mi - a
                        if c < 0:
                            continue
                        if c not in hw:
                            oh = c * CB + 8 * rr
                            hw[c] = [ar_s[z, j // 2, oh:oh + 8, (j % 2) * C:(j % 2 + 1) * C] for j in range(3, 6)]
                        hh = hw[c]
                        prods = (uu[2] * hh[0], uu[0] * hh[1], uu[1] * hh[2])
                        done += 1
                        for j in range(3):
                            acc[mi][j] = prods[j] if acc[mi][j] is None else acc[mi][j] + prods[j]
                res = [jnp.concatenate([x[0] - x[2], x[0] + x[1]], axis=1) for x in acc]
                base = rr * 64 + mb * ob * 4
                yb_u[base:base + ob * 4, :] = _pk(jnp.concatenate(res, axis=0))

    def inv(b):
        r0 = row0(b)
        y = jnp.dot(_up(yb_u[...]), _up(fi_s[...]), preferred_element_type=F32)
        cpt = T // C
        for rr in range(CB // 8):
            for m in range(NC):
                yp_s[m // cpt, pl.ds(r0 + 8 * rr, 8), (m % cpt) * C:(m % cpt + 1) * C] = (
                    y[rr * 128 + m * 8:rr * 128 + m * 8 + 8])

    def fold(x):
        for j in range(5):
            ls = slice(128 * j, min(128 * j + 128, D))
            w_ = ls.stop - ls.start
            sub = lax.broadcasted_iota(jnp.int32, (DH, 8, w_), 1)
            rt = {}
            res = []
            for t in range(4 * x, 4 * x + 5):
                if t == 4 and x == 0:
                    r = r4_s[:, ls]
                else:
                    r = lax.dot_general(_up(bd_u[:, t * 128:(t + 1) * 128]), wqkv_s[ls, t * 128:(t + 1) * 128],
                                        NT_DIMS, preferred_element_type=F32)
                    if t == 4:
                        r4_s[:, ls] = r
                rt[t] = r.reshape(DH, 8, w_)
                if t > 4 * x:
                    g = t - 1
                    w = jnp.where(sub <= 7 - g, rt[g], 0.0) + jnp.where(sub >= 7 - g, rt[g + 1], 0.0)
                    res.append(((w[:DH - 1] - w[DH - 1:]) * LOG2E).reshape(PR, w_))
                    if g % 2 == 1:
                        o = (g // 2) * PR
                        wt_u[o:o + PR, ls] = _pk(jnp.concatenate(res, axis=0))
                        res = []

    def feature_map(p, dst, g, is_q):
        ps = [p[8 * f:8 * f + 8] for f in range(DH - 1)]
        mx = jnp.maximum(_tree(jnp.maximum, ps), 0.0)
        mn = jnp.minimum(_tree(jnp.minimum, ps), 0.0)
        ep = [jnp.exp2(x - mx) for x in ps] + [jnp.exp2(-mx)]
        sp = _tree(jnp.add, ep)
        if not is_q:
            rp = _recip(sp)
            ep = [x * rp for x in ep]
        for j in range(9):
            dst[pl.ds(g * 144 + j, 8, stride=DH), :] = pltpu.pack_elementwise(
                [ep[2 * j], ep[2 * j + 1]], packed_dtype=BF16)
        if P['dep'] == 1:
            mn = jnp.minimum(mn, sp)
        elif P['dep'] == 2:
            mn = jnp.minimum(mn, ep[8])
        en = [jnp.exp2(mn - x) for x in ps] + [jnp.exp2(mn)]
        rn = _recip(_tree(jnp.add, en))
        if is_q:
            rn = rn * sp
        en = [x * rn for x in en]
        for j in range(9):
            dst[pl.ds(g * 144 + 9 + j, 8, stride=DH), :] = pltpu.pack_elementwise(
                [en[2 * j], en[2 * j + 1]], packed_dtype=BF16)

    def p_piece(x, gp, n, i, xt, buf=0):
        o = (2 * x + gp) * PR
        xn = xt[:, n * C:(n + 1) * C]
        dst = phik_u.at[buf, n] if x else phiq_u.at[i, n]
        if P['split']:
            pa = jnp.dot(_up(wt_u[o:o + 72, :]), xn, preferred_element_type=F32)
            feature_map(pa[:PR], dst, 2 * gp, not x)
            pb = jnp.dot(_up(wt_u[o + 72:o + PR, :]), xn, preferred_element_type=F32)
            feature_map(jnp.concatenate([pa[PR:], pb], axis=0), dst, 2 * gp + 1, not x)
        else:
            p = jnp.dot(_up(wt_u[o:o + PR, :]), xn, preferred_element_type=F32)
            feature_map(p[:PR], dst, 2 * gp, not x)
            feature_map(p[PR:], dst, 2 * gp + 1, not x)

    def v_part(j0, j1, n, xt, held, i, buf=0):
        o = 4 * PR + 4 * j0
        ex = 8 if j1 == D // 8 else 0
        vt = jnp.dot(_up(wt_u[o:o + 4 * (j1 - j0) + ex, :]), xt[:, n * C:(n + 1) * C], preferred_element_type=F32)
        if ex:
            g_s[i, :, n * C:(n + 1) * C] = jax.nn.sigmoid(vt[8 * (j1 - j0):8 * (j1 - j0) + 8])
        for j in range(j0, j1):
            held[j] = vt[8 * (j - j0):8 * (j - j0) + 8]
        sub = lax.broadcasted_iota(jnp.int32, (8, C), 0)
        for t in range(NF):
            if not (j0 < _W1[t] <= j1):
                continue
            rows = [held[j] for j in range(_W0[t], _W1[t])]
            if _LEAD[t]:
                rows[0] = jnp.where(sub < _LEAD[t], 1.0, rows[0])
            if _EXTRA[t]:
                rows.append(jnp.ones((8, C), F32))
            elif _TRAIL[t]:
                rows[-1] = jnp.where(sub >= 8 - _TRAIL[t], 1.0, rows[-1])
            vx_u.at[buf][_OFF[t] // 2:_OFF[t + 1] // 2, n * C:(n + 1) * C] = _pk(jnp.concatenate(rows, axis=0))

    def v_piece(hf, n, xt, held, i, buf=0):
        v_part(36 * hf, 36 * hf + 18, n, xt, held, i, buf)
        v_part(36 * hf + 18, 36 * hf + 36, n, xt, held, i, buf)

    def kv_acc(buf=0):
        for t in range(NF):
            ph = jnp.concatenate([_up(phik_u[buf, n, t * 64:(t + 1) * 64, :]) for n in range(2)], axis=1)
            r = lax.dot_general(_up(vx_u[buf, _OFF[t] // 2:_OFF[t + 1] // 2, :]), ph, NT_DIMS,
                                preferred_element_type=F32)
            if buf:
                acc_s[_OFF[t]:_OFF[t + 1], :] = r
            else:
                acc_s[_OFF[t]:_OFF[t + 1], :] += r

    def numer(i):
        sub = lax.broadcasted_iota(jnp.int32, (8, T), 0)
        omg = 1.0 - g_s[i]
        rs = []
        for t in range(NF):
            ph = jnp.concatenate([_up(phiq_u[i, n, t * 64:(t + 1) * 64, :]) for n in range(2)], axis=1)
            rs.append(jnp.dot(_up(kvm_u[_OFF[t] // 2:_OFF[t + 1] // 2, 0:128]), ph, preferred_element_type=F32))
        es = []
        for t in range(NF):
            first, last = rs[t][0:8], rs[t][_NR[t] - 8:]
            if _LEAD[t] and _TRAIL[t]:
                es.append(jnp.where(sub < _LEAD[t], first, last))
            else:
                es.append(first if _LEAD[t] else last)
        bc = {}
        for t in range(NF):
            den = es[t] if t == NF - 1 else es[t] + jnp.where(sub == _SPLIT[t], es[t + 1], 0.0)
            sc = omg * _recip(den)
            for h, s in _DEN[t].items():
                if t == 0 or h != _H0[t]:
                    bc[h] = jnp.broadcast_to(sc[s:s + 1], (8, T))
        outs = []
        for j in range(D // 8):
            parts = []
            for t in range(NF):
                if _W0[t] <= j < _W1[t]:
                    x = rs[t][8 * (j - _W0[t]):8 * (j - _W0[t]) + 8]
                    if j == _W0[t] and _LEAD[t]:
                        x = jnp.where(sub < _LEAD[t], 0.0, x)
                    if j == _W1[t] - 1 and _TRAIL[t] and not _EXTRA[t]:
                        x = jnp.where(sub >= 8 - _TRAIL[t], 0.0, x)
                    parts.append(x)
            num = parts[0] if len(parts) == 1 else parts[0] + parts[1]
            ha, hb = (8 * j) // DH, (8 * j + 7) // DH
            sc = bc[ha] if ha == hb else jnp.where(sub < DH * hb - 8 * j, bc[ha], bc[hb])
            outs.append(num * sc)
            if j % 18 == 17:
                ot_u.at[i][(j // 18) * 72:(j // 18 + 1) * 72, :] = _pk(jnp.concatenate(outs, axis=0))
                outs = []

    def final(sg, i):
        rs = slice(sg * 144, (sg + 1) * 144)
        bt = jnp.dot(_up(wot_u[sg * 72:(sg + 1) * 72, :]), _up(ot_u[i]), preferred_element_type=F32)
        qf = q_s[i, rs, :].astype(F32)
        ga = (qf.reshape(18, 8, T) * g_s[i][None]).reshape(144, T) * yp_s[i, rs, :]
        out_s[rs, i * T:(i + 1) * T] = (ga + bt).astype(BF16)

    def o_cp(sg, i0, i1, nsg):
        sl = (pl.ds(sg * 144, nsg * 144), pl.ds(i0 * T, (i1 - i0) * T))
        return cp(out_s.at[sl], out_h.at[sl], S_OUT)

    def div18(c):
        return (c * 3641) >> 16

    def wcol(rows):
        c = lax.broadcasted_iota(jnp.int32, (rows, 640), 1) + 512
        return jnp.where(c >= D, c - D, c)

    def hmask(lo, hi):
        col = lax.broadcasted_iota(jnp.int32, (8, hi - lo), 1) + lo
        return (div18(col) & 7) == lax.broadcasted_iota(jnp.int32, (8, hi - lo), 0)

    em = jnp.where(div18(wcol(H)) == lax.broadcasted_iota(jnp.int32, (H, 640), 0), 1.0, 0.0).astype(BF16)
    dmod = wcol(DH) - DH * div18(wcol(DH))
    wait(grp[0]())
    a_win = jnp.zeros((DH, 640), F32)
    for d in range(DH):
        rd = jnp.dot(wp_s[d], em, preferred_element_type=F32)
        a_win = jnp.where(dmod == d, rd, a_win)
    bd_u[:, 512:] = _pk(jnp.concatenate(
        [jnp.where(hmask(512, 2 * D), jnp.broadcast_to(a_win[f:f + 1], (8, 640)), 0.0) for f in range(DH)], axis=0))

    rows = [sh_s[j:j + 1, :].astype(F32) for j in range(4)]
    rows.append(dd_s[...].astype(F32).reshape(1, D))
    wt_u[4 * PR + D // 2:4 * PR + D // 2 + 8, :] = _pk(
        jnp.broadcast_to(gw_s[...].astype(F32).reshape(1, D), (16, D)))
    for j in range(5):
        tab_s[j] = jnp.broadcast_to(rows[j], (128, D)).T

    wait(grp[1]())
    a_q = pltpu.roll(a_win, D, 1)[:, :512]
    bd_u[:, :512] = _pk(jnp.concatenate(
        [jnp.where(hmask(0, 512), jnp.broadcast_to(a_q[f:f + 1], (8, 512)), 0.0) for f in range(DH)], axis=0))
    fold(1)

    wait(grp[2]())
    for i in range(2):
        xt = q_s[i]
        for gp in range(2):
            for n in range(2):
                p_piece(1, gp, n, i, xt, 1 - i)

    wait(grp[3]())
    shift_conv(0, _Clock(z_ref), 0, P['p3s1'])
    fold(0)
    for i in range(2):
        xt = q_s[i]
        for gp in range(2):
            for n in range(2):
                p_piece(0, gp, n, i, xt)

    wait(grp[4]())
    clk = _Clock(z_ref)
    fwd(0)
    shift_conv(1, clk, P['i1s0'], P['i1s1'])
    cmac(clk, P['i1c0'], P['i1c1'])
    wt_u[4 * PR:4 * PR + D // 2, :] = pltpu.bitcast(wqkv_s[:, 2 * D:3 * D].T, U32)
    for i in range(2):
        xt = q_s[i]
        for n in range(2):
            held = {}
            for hf in range(2):
                v_piece(hf, n, xt, held, i, 1 - i)
            if i == 1 and n == 0:
                kv_acc(1)

    def phase1(i, carry, do_inv=True):
        wait(g_loop(i))
        clk = _Clock(z_ref)
        fwd(i - 1)
        if do_inv:
            inv(i - 2)
        kv_acc()
        if not P['aft']:
            shift_conv(i, clk, P['s0'], P['s1'])
        cmac(clk, P['c0'], P['c1'], [(P['w0'] + j * P['wp'], P['w0'] + j * P['wp'] + P['wl']) for j in range(4)])
        if P['aft']:
            shift_conv(i, clk, P['s0'], P['s1'])
        xt = q_s[i]
        for n in range(2):
            held = {}
            for gp in range(2):
                if P['alt']:
                    p_piece(1, gp, n, i, xt)
                    v_part(36 * gp, 36 * gp + 18, n, xt, held, i)
                    p_piece(0, gp, n, i, xt)
                    v_part(36 * gp + 18, 36 * gp + 36, n, xt, held, i)
                else:
                    p_piece(1, gp, n, i, xt)
                    p_piece(0, gp, n, i, xt)
                    v_piece(gp, n, xt, held, i)
        return carry

    lax.fori_loop(2, NT, phase1, 0)
    if P['stop'] == 1:
        wait(grp[S_M1]() + grp[S_M2]())
        for r in (phiq_u, acc_s, yp_s, yb_u, g_s, phik_u, vx_u, ar_s):
            c = cp(r, r, S_OUT)

            @pl.when(z_ref[0] == 1)
            def _(c=c):
                c.start()
                c.wait()
        return

    wait(grp[S_M1]())
    clk = _Clock(z_ref)
    fwd(7)
    kv_acc()
    inv(6)
    shift_conv(8, clk, P['m1s0'], P['m1s1'])
    cmac(clk, P['m1c0'], P['m1c1'])
    wot_u[...] = pltpu.bitcast(wo_s[...].T, U32)
    kvm_u[:, 0:128] = _pk(acc_s[...] * msk_s[0] + msk_s[1])
    numer(0)
    for i in range(4):
        numer(i + 1)
        final(0, i)
        final(1, i)

    wait(grp[S_M2]())
    clk = _Clock(z_ref)
    fwd(8)
    inv(7)
    cmac(clk, P['m2c0'], P['m2c1'])
    o_cp(0, 0, 4, 2).start()
    for i in range(4, NT):
        if i + 1 < NT:
            numer(i + 1)
        final(0, i)
        final(1, i)

    o_cp(0, 0, 4, 2).wait()
    outs = [(0, 4, NT, 2)]
    o_cp(*outs[-1]).start()
    final(2, 0)
    inv(8)
    for sg, i in [(sg, i) for sg in (2, 3) for i in range(NT)][1:]:
        final(sg, i)
        if sg < 3 and i == NT - 1:
            outs.append((sg, 0, NT, 1))
            o_cp(*outs[-1]).start()
        elif sg == 3 and i in (3, 5, 6, 7):
            outs.append((sg, {3: 0, 5: 4, 6: 6, 7: 7}[i], i + 1, 1))
            o_cp(*outs[-1]).start()
    for o in outs:
        o_cp(*o).wait()


@jax.jit
def pallas_gated_mix__ssm_conv_h3__linear_kernel_hedgehog__prompt_kernel(A_q, A_k, A_v, A_shift_k, A_ssm_k, A_ssm_D, B_x, B_wqkv, B_w_phi, B_wo, gate_w):
    ins = (A_q[0].T, A_k[0].T, A_v[0].T, A_ssm_k, B_wqkv, B_wo, A_shift_k.T,
           B_w_phi.transpose(1, 2, 0), A_ssm_D, gate_w) + _consts()
    V = pltpu.VMEM
    scratch = [
        V((NT, D, T), BF16), V((NCB, CB, S), BF16), V((NCB, CB, S), BF16), V((NCB, CB, S), BF16),
        V((D, 3 * D), BF16), V((D, D), BF16),
        V((2, 4, NC * CB, 2 * C), F32), V((5, D, 128), F32), V((NC * CB // 2, 2 * C), U32),
        V((NT, D, T), F32), V((NT, 2, D, C), U32), V((2, 2, D, C), U32), V((NT, D // 2, T), U32),
        V((NT, 8, T), F32), V((D, S), BF16), V((NC * CB // 4, 2 * C), F32),
        V((72, 2 * D), U32), V((D // 2, D), U32), V((4 * PR + D // 2 + 8, D), U32),
        V((2, _OFF[NF] // 2, T), U32), V((_OFF[NF], 128), F32), V((_OFF[NF] // 2, 256), U32),
    ] + [V(x.shape, x.dtype) for x in ins[6:]] + [
        V((144, D), F32), pltpu.SMEM((8,), jnp.int32), pltpu.SemaphoreType.DMA((14,)),
    ]
    out = pl.pallas_call(
        _kernel,
        in_specs=[pl.BlockSpec(memory_space=pl.ANY)] * (len(ins) + 1),
        out_specs=pl.BlockSpec(memory_space=pl.ANY),
        out_shape=jax.ShapeDtypeStruct((D, S), BF16),
        scratch_shapes=scratch,
        compiler_params=pltpu.CompilerParams(vmem_limit_bytes=100 * 1024 * 1024),
        name="gm",
    )(np.zeros((8,), np.int32), *ins)
    return out.T[None]
```

```python
import functools
import numpy as np
import jax
import jax.numpy as jnp
from jax import lax
import jax.experimental.pallas as pl
import jax.experimental.pallas.tpu as pltpu


S, D, H, DH = 2048, 576, 32, 18
T = 256
NT = S // T
CB = 64
NCB = D // CB
C = 128
NC = S // C
NF = 9
PR = 17 * 8
LOG2E = float(np.log2(np.e))
EPS = 1e-6
RND = 1.002818
F32 = jnp.float32
BF16 = jnp.bfloat16
U32 = jnp.uint32
NT_DIMS = (((1,), (1,)), ((), ()))
HOP = 6
P = dict(c0=750, c1=4400, wr=20, ks=325, ke=400, qs=475, qe=475, tt0=200, tt1=700, drift=102, s0=550, s1=1750,
         ka0=100, ka1=550, p3s0=1000, p3s1=3875, i1c0=700, i1c1=3150, vf0=25, vf1=80, i1s0=1000, i1s1=1500,
         m1s0=2000, m1s1=4500, mac0=50, mac1=4400, mbc0=4500, mbc1=8900, bpos=2, wa0=2500, wa1=4500)
SEQ = 'Q0 V0 K0 Q1 V1 K1 Q2 Q3 V2 V3'

_H0 = [(128 * t) // 36 for t in range(NF)]
_H1 = [(128 * t + 127) // 36 for t in range(NF)]
_W0 = [(DH * h) // 8 for h in _H0]
_W1 = [-(-(DH * (h + 1)) // 8) for h in _H1]
_EXTRA = [(_W1[t] - _W0[t]) % 2 for t in range(NF)]
_NR = [8 * (_W1[t] - _W0[t] + _EXTRA[t]) for t in range(NF)]
_OFF = [sum(_NR[:t]) for t in range(NF + 1)]
_LEAD = [DH * _H0[t] - 8 * _W0[t] for t in range(NF)]
_TRAIL = [8 if _EXTRA[t] else 8 * _W1[t] - DH * (_H1[t] + 1) for t in range(NF)]
_SPLIT = [0, 1, 0, 1, 0, 1, 2, 3]


def _den_slots():
    slots = []
    for t in range(NF):
        free = list(range(_LEAD[t])) + list(range(8 - _TRAIL[t], 8))
        m = {}
        if t > 0:
            m[_H0[t]] = _SPLIT[t - 1]
        if t < NF - 1:
            m[_H1[t]] = _SPLIT[t]
        for s in m.values():
            free.remove(s)
        for h in range(_H0[t], _H1[t] + 1):
            if h not in m:
                m[h] = free.pop(0)
        slots.append(m)
    return slots


_DEN = _den_slots()
_ORD = [[0, _NR[t] // 8 - 1] + list(range(1, _NR[t] // 8 - 1)) for t in range(NF)]
_POS = [[o.index(j) for j in range(len(o))] for o in _ORD]
_PAIRS = ((0, 128, 64), (256, 96, 48), (448, 64, 64))


def _bf16_bits(x):
    u = np.ascontiguousarray(x, np.float32).view(np.uint32)
    return (u + 0x7FFF + ((u >> 16) & 1)) >> 16


def _pack_np(x):
    b = _bf16_bits(x)
    return (b[0::2] | (b[1::2] << 16)).astype(np.uint32)


def _consts():
    n = np.arange(C)[:, None].astype(np.float64)
    k = np.arange(C)[None, :].astype(np.float64)
    th = np.pi * (2 * k + 1) / (2 * C) * n
    f = np.concatenate([np.cos(th), -np.sin(th)], axis=1)
    finv = f.T / C
    mask = np.zeros((2, _OFF[NF], 128), np.float32)
    for t in range(NF):
        fi = 128 * t + np.arange(128)

        def row(r):
            return _OFF[t] + 8 * _POS[t][r // 8] + r % 8

        for r in range(_NR[t]):
            g = 8 * _W0[t] + r
            if DH * _H0[t] <= g < DH * (_H1[t] + 1):
                mask[0, row(r)] = (fi // 36 == g // DH)
        for h, s in _DEN[t].items():
            r = s if s < _LEAD[t] else _NR[t] - 8 + s
            mask[0, row(r)] = (fi // 36 == h)
            mask[1, row(r)] = EPS * ((fi // 36 == h) & (fi % 36 < DH))
    return _pack_np(f), _pack_np(finv), mask


def _recip(x, scale=1.0):
    r = pl.reciprocal(x, approx=True)
    return r * ((1.0 + scale) - x * r)


def _pack2(x, y):
    hi = pltpu.bitcast(y, U32) & jnp.uint32(0xFFFF0000)
    return lax.shift_right_logical(pltpu.bitcast(x, U32), jnp.uint32(16)) | hi


def _pk(x):
    return pltpu.bitcast(x.astype(BF16), U32)


def _up(x):
    return pltpu.bitcast(x, BF16)


def _mm(a, b):
    return jnp.dot(a, b, preferred_element_type=F32)


def _seq(op, xs):
    return functools.reduce(op, xs)


def _tree(op, xs):
    xs = list(xs)
    while len(xs) > 1:
        xs = [op(xs[i], xs[i + 1]) if i + 1 < len(xs) else xs[i] for i in range(0, len(xs), 2)]
    return xs[0]


def _warp(t0, t1, slow):
    ts = np.arange(t0, t1 + 1)
    rate = np.ones(len(ts))
    for a, b in slow:
        rate[(ts >= a) & (ts < b)] = P['wr'] / 100
    cum = np.cumsum(rate)
    return lambda fr: ts[min(int(np.searchsorted(cum, fr * cum[-1])), len(ts) - 1)]


class _Clock:
    def __init__(self, z_ref):
        self.z = z_ref
        self.v = [z_ref[0]]

    def at(self, t):
        n = int(t) // HOP
        while len(self.v) <= n:
            self.v.append(self.z[self.v[-1]])
        return self.v[n]


def _kernel(z_h, q_h, k_h, v_h, h_h, wqkv_h, wo_h, sh_h, wp_h, dd_h, gw_h, f_h, fi_h, msk_h,
            out_h,
            q_s, k_s, v_s, h_s, wqkv_s, wo_s, ara_s, arb_s, arc_s, ard_s, yb2_u, tab_s, yb_u, yp_s, phiq_u, phik_u, ot_u, g_s,
            out_s, ul_u, ts_u, tsb_u, wt2_u, wo2_u, ws_u, bd_u, wos_u, vx_u, acc_s, kvm_u,
            sh_s, wp_s, dd_s, gw_s, f_s, fi_s, msk_s, r4_s,
            z_ref, sem):
    wt_u = wt2_u.at[0]
    wot_u = wo2_u.at[0]
    ar_s = (ara_s, arb_s)
    ar2_s = (arc_s, ard_s)

    def cp(src, dst, s):
        return pltpu.make_async_copy(src, dst, sem.at[s])

    def q_cp(i, s):
        return [cp(q_h.at[:, pl.ds(i * T, T)], q_s.at[i], s)]

    def row_cp(src, dst, b, s):
        return [cp(src.at[pl.ds(b * CB, CB), :], dst.at[b], s)]

    def kv_cp(b, s):
        return row_cp(k_h, k_s, b, s) + row_cp(v_h, v_s, b, s)

    def w_cp(lo, hi, s):
        return [cp(wqkv_h.at[:, pl.ds(lo, hi - lo)], wqkv_s.at[:, pl.ds(lo, hi - lo)], s)]

    S_LOOP, S_M1, S_M2, S_OUT = 3, 11, 12, 13
    grp = {
        0: lambda: [cp(a, b, 0) for a, b in ((wp_h, wp_s), (sh_h, sh_s), (dd_h, dd_s), (gw_h, gw_s), (z_h, z_ref))],
        1: lambda: w_cp(512, 1152, 1),
        2: lambda: q_cp(0, 2) + q_cp(1, 2),
        3: lambda: w_cp(0, 512, 3) + kv_cp(0, 3) + [cp(f_h, f_s, 3)] + row_cp(h_h, h_s, 0, 3),
        4: lambda: w_cp(1152, 1728, 4) + kv_cp(1, 4) + [cp(fi_h, fi_s, 4)],
        S_M1: lambda: row_cp(h_h, h_s, 7, S_M1) + kv_cp(8, S_M1) + [cp(wo_h, wo_s, S_M1), cp(msk_h, msk_s, S_M1)],
        S_M2: lambda: row_cp(h_h, h_s, 8, S_M2),
    }

    def g_loop(i):
        return q_cp(i, S_LOOP + i) + row_cp(h_h, h_s, i - 1, S_LOOP + i) + kv_cp(i, S_LOOP + i)

    def o_cp(r0, r1, i0, i1):
        sl = (pl.ds(r0, r1 - r0), pl.ds(i0 * T, (i1 - i0) * T))
        return cp(out_s.at[sl], out_h.at[sl], S_OUT)

    for g in range(5):
        for c in grp[g]():
            c.start()
    for i in range(2, NT):
        for c in g_loop(i):
            c.start()
    for g in (S_M1, S_M2):
        for c in grp[g]():
            c.start()

    def wait(cs):
        for c in cs:
            c.wait()

    def row0(b):
        return b * CB if isinstance(b, int) else pl.multiple_of(b * CB, CB)

    def shift_conv(b, clk, t0, t1):
        lane = lax.broadcasted_iota(jnp.int32, (8, C), 1)
        m1 = lane < C - 1
        m2 = lane < C - 2
        r0 = row0(b)
        zf = z_ref[1].astype(F32)
        for rr in range(CB // 8):
            tp = None
            p1 = p2 = None
            for aq in range(NC // 4):
                z = clk.at(t0 + (t1 - t0) * (rr * 4 + aq) / 32)
                if tp is None:
                    tp = [tab_s[j + z, pl.ds(r0 + 8 * rr, 8), :] for j in range(4)]
                kk = k_s[b + z, 8 * rr:8 * rr + 8, aq * 4 * C:(aq + 1) * 4 * C].astype(F32)
                vv = v_s[b + z, 8 * rr:8 * rr + 8, aq * 4 * C:(aq + 1) * 4 * C].astype(F32)
                us = []
                for hf in range(4):
                    ka = kk[:, hf * C:(hf + 1) * C]
                    s1 = pltpu.roll(jnp.where(m1, ka, 0.0 if p1 is None else p1) + zf, 1, 1)
                    p1 = ka
                    aa = tp[0] * ka + tp[1] * s1
                    bb = tp[2] * ka + tp[3] * s1
                    s2 = pltpu.roll(jnp.where(m2, bb, 0.0 if p2 is None else p2), 2, 1)
                    p2 = bb
                    us.append((aa + s2) * vv[:, hf * C:(hf + 1) * C])
                o = (rr * (NC // 4) + aq) * 8
                uu = jnp.concatenate([jnp.concatenate([us[0], us[2]], axis=1),
                                      jnp.concatenate([us[1], us[3]], axis=1)], axis=0)
                ul_u[o:o + 8, :] = _pk(uu)

    def fwd(b, ar_s=ar_s, do_u=True, do_h=True, anchor=False):
        lane = lax.broadcasted_iota(jnp.int32, (8, C), 1)
        sgn = jnp.where((lane & 1) == 0, 1.0, -1.0).astype(F32)
        r0 = row0(b)
        hc = CB // 2
        n = NC * hc
        fm = _up(f_s[...])
        for hf in range(2):
            ar = ar_s[hf]
            if do_u:
                ul = _up(ul_u[hf * 128:(hf + 1) * 128, :])
                r = _mm(jnp.concatenate([ul[:, :C], ul[:, C:]], axis=0), fm)
                ar[0, 0, :, 0:2 * C] = r
                if anchor and hf == 0:
                    q_s[NT, 0:16, :] = r[0:16].astype(BF16)
                ar[0, 0, :, 2 * C:] = r[:, :C] + r[:, C:]
            if do_h:
                hb = h_s[b, hf * hc:(hf + 1) * hc, :]
                r = _mm(jnp.concatenate([hb[:, a * C:(a + 1) * C] for a in range(NC)], axis=0), fm)
                hre, him = r[:, :C], r[:, C:]
                sg = jnp.tile(sgn, ((n - hc) // 8, 1))
                re = jnp.concatenate([hre[:hc] + tab_s[4, pl.ds(r0 + hf * hc, hc), :],
                                      hre[hc:] - sg * him[:n - hc]], axis=0)
                im = jnp.concatenate([him[:hc], him[hc:] + sg * hre[:n - hc]], axis=0)
                ar[0, 1, :, 2 * C:] = re
                ar[0, 1, :, 0:C] = im - re
                ar[0, 1, :, C:2 * C] = im + re

    def cmac(clk, t0, t1, slow=(), ar_s=ar_s, yb_u=yb_u, extras=()):
        extras = list(extras)
        tm = _warp(t0, t1, slow)
        total = (CB // 8) * 136
        done = 0
        for rr in range(CB // 8):
            for mb in range(NC // 2):
                acc = [None, None]
                hw = {}
                for a in range(2 * mb + 2):
                    z = clk.at(tm(done / total))
                    while extras and extras[0][0] <= done / total:
                        extras.pop(0)[1](z)
                    o = (a % 4 // 2) * 256 + ((rr % 4 * 4 + a // 4) * 2 + a % 2) * 8
                    uu = ar_s[rr // 4][z, 0, o:o + 8, :]
                    for mi in range(2):
                        c = 2 * mb + mi - a
                        if c < 0:
                            continue
                        if c not in hw:
                            oh = c * 32 + 8 * (rr % 4)
                            hw[c] = ar_s[rr // 4][z, 1, oh:oh + 8, :]
                        prod = uu * hw[c]
                        done += 1
                        acc[mi] = prod if acc[mi] is None else acc[mi] + prod
                res = [jnp.concatenate([x[:, 2 * C:] - x[:, C:2 * C], x[:, 2 * C:] + x[:, :C]], axis=1) for x in acc]
                base = rr * 64 + mb * 8
                yb_u[base:base + 8, :] = _pk(jnp.concatenate(res, axis=0))

    def inv(b, yb_u=yb_u, parts=range(4)):
        r0 = row0(b)
        cpt = T // C
        for pt in parts:
            y = _mm(_up(yb_u[pt * 128:(pt + 1) * 128, :]), _up(fi_s[...]))
            for r2 in range(2):
                rr = 2 * pt + r2
                for m in range(NC):
                    yp_s[m // cpt, pl.ds(r0 + 8 * rr, 8), (m % cpt) * C:(m % cpt + 1) * C] = (
                        y[r2 * 128 + m * 8:r2 * 128 + m * 8 + 8])

    def fold(x):
        for j in range(5):
            ls = slice(128 * j, min(128 * j + 128, D))
            w_ = ls.stop - ls.start
            sub = lax.broadcasted_iota(jnp.int32, (DH, 8, w_), 1)
            rt = {}
            res = []
            for t in range(4 * x, 4 * x + 5):
                if t == 4 and x == 0:
                    r = r4_s[:, ls]
                else:
                    cuts = (0, 16, 40, 56, 72) if (t, j) == (8, 4) else (0, 72)
                    r = jnp.concatenate([
                        lax.dot_general(_up(bd_u[a:b, t * 128:(t + 1) * 128]), wqkv_s[ls, t * 128:(t + 1) * 128],
                                        NT_DIMS, preferred_element_type=F32)
                        for a, b in zip(cuts, cuts[1:])], axis=0)
                    if t == 4:
                        r4_s[:, ls] = r
                rt[t] = r.reshape(DH, 8, w_)
                if t > 4 * x:
                    g = t - 1
                    w = jnp.where(sub <= 7 - g, rt[g], 0.0) + jnp.where(sub >= 7 - g, rt[g + 1], 0.0)
                    res.append(((w[:DH - 1] - w[DH - 1:]) * LOG2E).reshape(PR, w_))
                    if g % 2 == 1:
                        o = (g // 2) * PR
                        wt_u[o:o + PR, ls] = _pk(jnp.concatenate(res, axis=0))
                        res = []

    def feature_map(p, dst, g, is_q, fast=False):
        red = _tree if fast else _seq
        ps = [p[8 * f:8 * f + 8] for f in range(DH - 1)]
        mx = jnp.maximum(red(jnp.maximum, ps), 0.0)
        mn = jnp.minimum(red(jnp.minimum, ps), 0.0)
        if is_q:
            mx = mx - float(np.log2(RND))
        ep = [jnp.exp2(x - mx) for x in ps] + [jnp.exp2(-mx)]
        sp = red(jnp.add, ep)
        if not is_q:
            rp = _recip(sp, RND)
            ep = [x * rp for x in ep]
        for j in range(9):
            dst[pl.ds(g * 144 + j, 8, stride=DH), :] = _pack2(ep[2 * j], ep[2 * j + 1])
        if not fast:
            mn = jnp.minimum(mn, sp)
        en = [jnp.exp2(mn - x) for x in ps] + [jnp.exp2(mn)]
        sn = red(jnp.add, en)
        rn = _recip(sn) * sp if is_q else _recip(sn, RND)
        en = [x * rn for x in en]
        for j in range(9):
            dst[pl.ds(g * 144 + 9 + j, 8, stride=DH), :] = _pack2(en[2 * j], en[2 * j + 1])

    def p_piece(x, gp, n, i, xt, buf=0, fast=False):
        o = (2 * x + gp) * PR
        dst = phik_u.at[buf, n] if x else phiq_u.at[i, n]
        p = _mm(_up(wt_u[o:o + PR, :]), xt[:, n * C:(n + 1) * C])
        feature_map(p[:PR], dst, 2 * gp, not x)
        feature_map(p[PR:], dst, 2 * gp + 1, not x, fast)

    def v_emit(n, held, buf=0):
        sub = lax.broadcasted_iota(jnp.int32, (8, C), 0)
        done = held.setdefault('done', set())
        for t in range(NF):
            if t in done or not all(j in held for j in range(_W0[t], _W1[t])):
                continue
            done.add(t)
            rows = [held[j] for j in range(_W0[t], _W1[t])]
            if _LEAD[t]:
                rows[0] = jnp.where(sub < _LEAD[t], 1.0, rows[0])
            if _EXTRA[t]:
                rows.append(jnp.ones((8, C), F32))
            elif _TRAIL[t]:
                rows[-1] = jnp.where(sub >= 8 - _TRAIL[t], 1.0, rows[-1])
            vx_u.at[buf][_OFF[t] // 2:_OFF[t + 1] // 2, n * C:(n + 1) * C] = _pk(
                jnp.concatenate([rows[j] for j in _ORD[t]], axis=0))

    def v_part(j0, j1, n, xt, held, i, buf=0, gate=True):
        o = 4 * PR + 4 * j0
        ex = 8 if j1 == D // 8 and gate else 0
        vt = _mm(_up(wt_u[o:o + 4 * (j1 - j0) + ex, :]), xt[:, n * C:(n + 1) * C])
        if ex:
            g_s[i, :, n * C:(n + 1) * C] = jax.nn.sigmoid(vt[8 * (j1 - j0):8 * (j1 - j0) + 8])
        for j in range(j0, j1):
            held[j] = vt[8 * (j - j0):8 * (j - j0) + 8]
        v_emit(n, held, buf)

    def a_step(top, bot, dst, lh, z, w2_u=wt2_u, ws_u=ws_u):
        def ld(r, o):
            return _up(w2_u[z, r:r + 8, o + lh * C:o + (lh + 1) * C]).astype(F32)

        a11, a12, a21, a22 = ld(top, 0), ld(top, 256), ld(bot, 0), ld(bot, 256)
        for m, x in enumerate((a11 + a22, a21 + a22, a11 + a12, a21 - a11, a12 - a22)):
            ws_u[dst:dst + 8, m * 256 + lh * C:m * 256 + (lh + 1) * C] = _pk(x)

    def t_step(i, r, z):
        b1 = q_s[i + z, 16 * r:16 * r + 16, :].astype(F32)
        b2 = q_s[i + z, 256 + 16 * r:256 + 16 * r + 16, :].astype(F32)
        b11, b12, b21, b22 = b1[:, :C], b1[:, C:], b2[:, :C], b2[:, C:]
        slabs = ((b11 + b22, b11), (b12 - b22, b21 - b11), (b22, b11 + b12), (b21 + b22, b12))
        for sl, pr in enumerate(slabs):
            ts_u[sl * 128 + 8 * r:sl * 128 + 8 * r + 8, :] = _pk(jnp.concatenate(pr, axis=1))
        tsb_u[8 * r:8 * r + 8, 0:C] = _pk(b21)

        def gw(o):
            return jnp.tile(tab_s[5, o:o + 16, :], (1, 2))

        gl = b1 * gw(16 * r) + b2 * gw(256 + 16 * r)
        if r % 4 == 0:
            o = 512 + 4 * r
            gl = gl + q_s[i + z, o:o + 16, :].astype(F32) * gw(o)
        return gl

    def s_piece(top, bot, srow, nr, xt, sink):
        def tb(m):
            return _up(ts_u[(m // 2) * 128:(m // 2 + 1) * 128, (m % 2) * C:(m % 2 + 1) * C])

        def sa(m):
            return _up(ws_u[srow:srow + nr, m * 256:(m + 1) * 256])

        def tail(r, n):
            return _mm(_up(wt_u[r:r + nr, 512:D]), xt[512:D, n * C:(n + 1) * C])

        m3 = _mm(_up(wt_u[top:top + nr, 0:256]), tb(2))
        m5 = _mm(sa(2), tb(4))
        sink(0, 1, m3 + m5 + tail(top, 1))
        m2 = _mm(sa(1), tb(1))
        m4 = _mm(_up(wt_u[bot:bot + nr, 256:512]), tb(3))
        sink(1, 0, m2 + m4 + tail(bot, 0))
        m1 = _mm(sa(0), tb(0))
        sink(0, 0, (m4 - m5) + m1 + _mm(sa(4), tb(6)) + tail(top, 0))
        sink(1, 1, (m3 - m2) + m1 + _mm(sa(3), tb(5)) + tail(bot, 1))

    def ks_piece(part, xt, keep):
        lo, nr = ((0, 72), (72, 64))[part]

        def sink(half, n, p):
            dst = phik_u.at[0, n]
            if part == 0:
                feature_map(p[:PR], dst, 2 * half, False)
                keep[half, n] = p[PR:]
            else:
                feature_map(jnp.concatenate([keep[half, n], p], axis=0), dst, 2 * half + 1, False)

        s_piece(2 * PR + lo, 3 * PR + lo, lo, nr, xt, sink)

    def vs_piece(q4, xt, helds):
        top = (q4 // 2) * 128 + (q4 % 2) * 32

        def sink(half, n, v):
            j0 = (top + 64 * half) // 4
            for j in range(8):
                helds[n][j0 + j] = v[8 * j:8 * j + 8]
            v_emit(n, helds[n])

        s_piece(4 * PR + top, 4 * PR + top + 64, PR + 32 * q4, 32, xt, sink)

    def kv_acc(buf=0):
        for t in range(NF):
            ph = jnp.concatenate([_up(phik_u[buf, n, t * 64:(t + 1) * 64, :]) for n in range(2)], axis=1)
            r = lax.dot_general(_up(vx_u[buf, _OFF[t] // 2:_OFF[t + 1] // 2, :]), ph, NT_DIMS,
                                preferred_element_type=F32)
            if buf:
                acc_s[_OFF[t]:_OFF[t + 1], :] = r
            else:
                acc_s[_OFF[t]:_OFF[t + 1], :] += r

    def numer(i):
        sub = lax.broadcasted_iota(jnp.int32, (8, T), 0)
        omg = 1.0 - g_s[i]
        rs = []
        for t in range(NF):
            ph = jnp.concatenate([_up(phiq_u[i, n, t * 64:(t + 1) * 64, :]) for n in range(2)], axis=1)
            rs.append(_mm(_up(kvm_u[_OFF[t] // 2:_OFF[t + 1] // 2, 0:128]), ph))
        es = []
        for t in range(NF):
            first, last = rs[t][0:8], rs[t][8:16]
            if _LEAD[t] and _TRAIL[t]:
                es.append(jnp.where(sub < _LEAD[t], first, last))
            else:
                es.append(first if _LEAD[t] else last)
        bc = {}
        for t in range(NF):
            den = es[t] if t == 0 else es[t] + jnp.where(sub == _SPLIT[t - 1], es[t - 1], 0.0)
            sc = omg * _recip(den)
            for h, s in _DEN[t].items():
                if t == NF - 1 or h != _H1[t]:
                    bc[h] = jnp.broadcast_to(sc[s:s + 1], (8, T))
        outs = []
        for j in range(D // 8):
            parts = []
            for t in range(NF):
                if _W0[t] <= j < _W1[t]:
                    o = 8 * _POS[t][j - _W0[t]]
                    x = rs[t][o:o + 8]
                    if j == _W0[t] and _LEAD[t]:
                        x = jnp.where(sub < _LEAD[t], 0.0, x)
                    if j == _W1[t] - 1 and _TRAIL[t] and not _EXTRA[t]:
                        x = jnp.where(sub >= 8 - _TRAIL[t], 0.0, x)
                    parts.append(x)
            num = parts[0] if len(parts) == 1 else parts[0] + parts[1]
            ha, hb = (8 * j) // DH, (8 * j + 7) // DH
            sc = bc[ha] if ha == hb else jnp.where(sub < DH * hb - 8 * j, bc[ha], bc[hb])
            outs.append(num * sc)
            if j < 64 and j % 4 == 3:
                b1 = jnp.concatenate(outs[0:2], axis=0)
                b2 = jnp.concatenate(outs[2:4], axis=0)
                b11, b12, b21, b22 = b1[:, :C], b1[:, C:], b2[:, :C], b2[:, C:]
                slabs = ((b11 + b22, b11), (b12 - b22, b21 - b11), (b22, b11 + b12))
                o = (j // 4) * 8
                for sl, pr in enumerate(slabs):
                    ot_u.at[i][sl * 128 + o:sl * 128 + o + 8, :] = _pk(jnp.concatenate(pr, axis=1))
                ot_u.at[i][384 + o:384 + o + 8, 0:C] = _pk(b21 + b22)
                outs = []
        ot_u.at[i][512:544, :] = _pk(jnp.concatenate(outs, axis=0))

    def prep_wo(clk):
        wo = wo_s[...]
        wp_ = jnp.concatenate([wo[32 * g:32 * g + 16] for g in range(16)]
                              + [wo[32 * g + 16:32 * g + 32] for g in range(16)] + [wo[512:]], axis=0)
        wot_u[...] = pltpu.bitcast(wp_.T, U32)
        steps = [(r0 // 2 + r, (r0 + nr) // 2 + r, r0 // 4 + r, lh)
                 for r0, nr, _ in _PAIRS for r in range(0, nr // 2, 8) for lh in range(2)]
        for j, st in enumerate(steps):
            a_step(*st, clk.at(P['wa0'] + (P['wa1'] - P['wa0']) * j / len(steps)), wo2_u, wos_u)

    def final(p, i):
        r0, nr, step = _PAIRS[p]
        gate = g_s[i]
        bs = [_up(ot_u[i, (m // 2) * 128:(m // 2 + 1) * 128, (m % 2) * C:(m % 2 + 1) * C]) for m in range(7)]
        bt = _up(ot_u[i, 512:544, :])
        for lo in range(0, nr, step):
            hi = lo + step
            ws = slice(r0 // 4 + lo // 2, r0 // 4 + hi // 2)
            top = slice((r0 + lo) // 2, (r0 + hi) // 2)
            bot = slice((r0 + nr + lo) // 2, (r0 + nr + hi) // 2)
            sa = [wos_u[ws, m * 256:(m + 1) * 256] for m in range(5)]
            lhs = (sa[0], sa[1], wot_u[top, 0:256], wot_u[bot, 256:512], sa[2], sa[3], sa[4])
            mm = [_mm(_up(lhs[m]), bs[m]) for m in range(7)]
            tt = _mm(_up(wot_u[top, 512:D]), bt)
            tb = _mm(_up(wot_u[bot, 512:D]), bt)
            ctop = jnp.concatenate([mm[0] + mm[3] - mm[4] + mm[6], mm[2] + mm[4]], axis=1) + tt
            cbot = jnp.concatenate([mm[1] + mm[3], mm[0] - mm[1] + mm[2] + mm[5]], axis=1) + tb
            for half, cc in ((0, ctop), (1, cbot)):
                rs = slice(r0 + nr * half + lo, r0 + nr * half + hi)
                qf = q_s[i, rs, :].astype(F32)
                ga = (qf.reshape((hi - lo) // 8, 8, T) * gate[None]).reshape(hi - lo, T) * yp_s[i, rs, :]
                out_s[rs, i * T:(i + 1) * T] = (ga + cc).astype(BF16)

    def div18(c):
        return (c * 3641) >> 16

    def wcol(rows):
        c = lax.broadcasted_iota(jnp.int32, (rows, 640), 1) + 512
        return jnp.where(c >= D, c - D, c)

    def hmask(lo, hi):
        col = lax.broadcasted_iota(jnp.int32, (8, hi - lo), 1) + lo
        return (div18(col) & 7) == lax.broadcasted_iota(jnp.int32, (8, hi - lo), 0)

    em = jnp.where(div18(wcol(H)) == lax.broadcasted_iota(jnp.int32, (H, 640), 0), 1.0, 0.0).astype(BF16)
    dmod = wcol(DH) - DH * div18(wcol(DH))
    wait(grp[0]())
    a_win = jnp.zeros((DH, 640), F32)
    for d in range(DH):
        a_win = jnp.where(dmod == d, _mm(wp_s[d], em), a_win)
    bd_u[:, 512:] = _pk(jnp.concatenate(
        [jnp.where(hmask(512, 2 * D), jnp.broadcast_to(a_win[f:f + 1], (8, 640)), 0.0) for f in range(DH)], axis=0))

    rows = [sh_s[j:j + 1, :].astype(F32) for j in range(4)]
    rows.append(dd_s[...].astype(F32).reshape(1, D))
    wt_u[4 * PR + D // 2:4 * PR + D // 2 + 8, :] = _pk(
        jnp.broadcast_to(gw_s[...].astype(F32).reshape(1, D), (16, D)))
    rows.append(gw_s[...].astype(F32).reshape(1, D))
    for j in range(6):
        tab_s[j] = jnp.broadcast_to(rows[j], (128, D)).T

    wait(grp[1]())
    a_q = pltpu.roll(a_win, D, 1)[:, :512]
    bd_u[:, :512] = _pk(jnp.concatenate(
        [jnp.where(hmask(0, 512), jnp.broadcast_to(a_q[f:f + 1], (8, 512)), 0.0) for f in range(DH)], axis=0))
    fold(1)

    wait(grp[2]())
    clk = _Clock(z_ref)
    for r2 in range(PR // 4):
        r = r2 // 2 * 8
        a_step(2 * PR + r, 3 * PR + r, r, r2 % 2, clk.at(P['ka0'] + (P['ka1'] - P['ka0']) * r2 * 4 / PR))
    for i in range(2):
        xt = q_s[i]
        for gp in range(2):
            for n in range(2):
                p_piece(1, gp, n, i, xt, 1 - i, (i, gp, n) == (1, 1, 1))

    wait(grp[3]())
    shift_conv(0, _Clock(z_ref), P['p3s0'], P['p3s1'])
    fold(0)
    for i in range(2):
        xt = q_s[i]
        for gp in range(2):
            for n in range(2):
                p_piece(0, gp, n, i, xt)
    fwd(0, do_u=False)

    wait(grp[4]())
    clk = _Clock(z_ref)
    fwd(0, do_h=False)
    shift_conv(1, clk, P['i1s0'], P['i1s1'])
    wt_u[4 * PR:4 * PR + D // 2, :] = pltpu.bitcast(wqkv_s[:, 2 * D:3 * D].T, U32)
    ex = []
    for r2 in range(32):
        r = r2 // 2
        o = 4 * PR + (r // 8) * 128 + (r % 8) * 8
        ex.append(((P['vf0'] + (P['vf1'] - P['vf0']) * r2 / 32) / 100,
                   functools.partial(a_step, o, o + 64, PR + 8 * r, r2 % 2)))
    cmac(clk, P['i1c0'], P['i1c1'], extras=ex)
    for i in range(2):
        xt = q_s[i]
        for n in range(2):
            held = {}
            for j in ((3, 2, 1, 0) if (i, n) == (1, 1) else range(4)):
                v_part(18 * j, 18 * j + 18, n, xt, held, i, 1 - i)
            if i == 1 and n == 0:
                kv_acc(1)

    def phase1(i, carry):
        wait(g_loop(i))
        clk = _Clock(z_ref)
        fwd(i - 1, anchor=True)
        gl = _seq(jnp.add, [t_step(i, r, clk.at(P['tt0'] + (P['tt1'] - P['tt0']) * r / 16)) for r in range(16)])
        gl = gl[:8] + gl[8:]
        gl = gl + pltpu.roll(gl, 4, 0)
        gl = gl + pltpu.roll(gl, 2, 0)
        gl = gl + pltpu.roll(gl, 1, 0)
        g_s[i] = jax.nn.sigmoid(gl)
        inv(i - 2)
        kv_acc()
        shift_conv(i, clk, P['s0'], P['s1'])
        t, slow = 1960, []
        for tok in SEQ.split():
            d = dict(K0=648, K1=576, V=288, Q=340)[tok if tok[0] == 'K' else tok[0]] * P['drift'] // 100
            if tok[0] == 'K':
                slow.append((t + P['ks'], t + d + P['ke']))
            if tok[0] == 'Q':
                slow.append((t + P['qs'], t + d + P['qe']))
            t += d
        cmac(clk, P['c0'], P['c1'], slow)
        xt = jnp.concatenate([
            jnp.concatenate([_up(ts_u[0:128, C:]), _up(ts_u[384:512, C:])], axis=1),
            jnp.concatenate([_up(tsb_u[0:128, 0:C]), _up(ts_u[256:384, 0:C])], axis=1),
            q_s[i, 512:D, :]], axis=0)
        helds = ({}, {})
        keep = {}
        for tok in SEQ.split():
            x = int(tok[1:])
            if tok[0] == 'K':
                ks_piece(x, xt, keep)
            elif tok[0] == 'V':
                vs_piece(x, xt, helds)
            else:
                p_piece(0, x % 2, x // 2, i, xt)
        for n in range(2):
            v_part(64, 72, n, xt, helds[n], i, gate=False)
        return carry

    lax.fori_loop(2, NT, phase1, 0)

    wait(grp[S_M1]())
    clk = _Clock(z_ref)
    inv(6, parts=(0, 1))
    kv_acc()
    fwd(7)
    prep_wo(clk)
    shift_conv(8, clk, P['m1s0'], P['m1s1'])
    kvm_u[:, 0:128] = _pk(jnp.where(msk_s[0] > 0, acc_s[...], 0.0) + msk_s[1])
    for i in range(NT):
        numer(i)
    inv(6, parts=(2, 3))

    wait(grp[S_M2]())
    clk = _Clock(z_ref)
    cmac(clk, P['mac0'], P['mac1'])
    for i in range(NT):
        if i == P['bpos']:
            fwd(8, ar2_s)
            cmac(clk, P['mbc0'], P['mbc1'], (), ar2_s, yb2_u)
        final(0, i)
    o_cp(0, 256, 0, NT).start()
    for i in range(NT):
        final(1, i)

    o_cp(0, 256, 0, NT).wait()
    outs = [(256, 448, 0, NT)]
    o_cp(*outs[-1]).start()
    inv(7)
    inv(8, yb2_u)
    for i in range(NT):
        final(2, i)
        if i in (3, 5, 6, 7):
            outs.append((448, D, {3: 0, 5: 4, 6: 6, 7: 7}[i], i + 1))
            o_cp(*outs[-1]).start()
    for o in outs:
        o_cp(*o).wait()


@jax.jit
def pallas_gated_mix__ssm_conv_h3__linear_kernel_hedgehog__prompt_kernel(A_q, A_k, A_v, A_shift_k, A_ssm_k, A_ssm_D, B_x, B_wqkv, B_w_phi, B_wo, gate_w):
    ins = (A_q[0].T, A_k[0].T, A_v[0].T, A_ssm_k, B_wqkv, B_wo, A_shift_k.T,
           B_w_phi.transpose(1, 2, 0), A_ssm_D, gate_w) + _consts()
    V = pltpu.VMEM
    scratch = [
        V((NT + 1, D, T), BF16), V((NCB, CB, S), BF16), V((NCB, CB, S), BF16), V((NCB, CB, S), BF16),
        V((D, 3 * D), BF16), V((D, D), BF16),
        V((2, 2, 512, 3 * C), F32), V((2, 2, 512, 3 * C), F32), V((2, 2, 512, 3 * C), F32),
        V((2, 2, 512, 3 * C), F32), V((NC * CB // 2, 2 * C), U32),
        V((6, D, 128), F32), V((NC * CB // 2, 2 * C), U32),
        V((NT, D, T), F32), V((NT, 2, D + 32, C), U32), V((2, 2, D + 32, C), U32), V((NT, 544, T), U32),
        V((NT, 8, T), F32), V((D, S), BF16), V((NC * CB // 4, 2 * C), U32), V((512, T), U32), V((128, T), U32),
        V((2, 864, D), U32), V((2, D // 2, D), U32), V((PR + 128, 5 * 256), U32), V((72, 2 * D), U32),
        V((144, 5 * 256), U32),
        V((2, _OFF[NF] // 2, T), U32), V((_OFF[NF], 128), F32), V((_OFF[NF] // 2, 256), U32),
    ] + [V(x.shape, x.dtype) for x in ins[6:]] + [
        V((144, D), F32), pltpu.SMEM((8,), jnp.int32), pltpu.SemaphoreType.DMA((14,)),
    ]
    out = pl.pallas_call(
        _kernel,
        in_specs=[pl.BlockSpec(memory_space=pl.ANY)] * (len(ins) + 1),
        out_specs=pl.BlockSpec(memory_space=pl.ANY),
        out_shape=jax.ShapeDtypeStruct((D, S), BF16),
        scratch_shapes=scratch,
        compiler_params=pltpu.CompilerParams(vmem_limit_bytes=100 * 1024 * 1024),
        name="gm",
    )(np.zeros((8,), np.int32), *ins)
    return out.T[None]
```
